```python
import jax
import jax.numpy as jnp

def _softmax(x, axis=-1):
    return jax.nn.softmax(x, axis=axis)
def _gelu(x):
    return jax.nn.gelu(x, approximate=True)
def _silu(x):
    return jax.nn.silu(x)
def _sigmoid(x):
    return jax.nn.sigmoid(x)
def _layernorm(x, axis=-1, eps=1e-5):
    m = jnp.mean(x, axis=axis, keepdims=True)
    v = jnp.var(x, axis=axis, keepdims=True)
    return (x - m) / jnp.sqrt(v + eps)
def _scatter_add(tgt, idx, src, axis=0):
    return tgt.at[idx].add(src)
def _segment_sum(src, seg, n):
    return jax.ops.segment_sum(src, seg, n)
class _Rng:
    def __init__(self, key):
        self._k = key
    def _next(self):
        self._k, sub = jax.random.split(self._k)
        return sub
    def normal(self, shape):
        return jax.random.normal(self._next(), shape, dtype=jnp.bfloat16)
    def randint(self, lo, hi, shape):
        return jax.random.randint(self._next(), shape, lo, hi, dtype=jnp.int32)
    def uniform(self, shape, lo=0.0, hi=1.0):
        return jax.random.uniform(self._next(), shape, jnp.bfloat16, lo, hi)
    def permutation(self, n):
        return jax.random.permutation(self._next(), n)


kernel_name = 'recurrent_scan__compressed_kv_cla__dense_activation_gelu__decode'

def setup_inputs():
    _rng = _Rng(jax.random.key(int.from_bytes(__import__("os").urandom(4), "little")))
    _w = (lambda a: (lambda t: t.astype(jnp.bfloat16) if jnp.issubdtype(t.dtype, jnp.floating) else t)(jnp.asarray(a)))
    def _A_setup():
        B, H, Sq, Sk, D, M = 2, 32, 1, 16384, 128, 512
        Dc = 4 * D
        return {
            "x": _w((lambda *s: _rng.normal(s) * 0.05)(B, Sq, M)),
            "c_kv": _w((lambda *s: _rng.normal(s) * 0.05)(B, Sk, Dc)),
            "w_q": _w((lambda *s: _rng.normal(s) * 0.05)(M, H, D) * (M ** -0.5)),
            "w_uk": _w((lambda *s: _rng.normal(s) * 0.05)(Dc, H, D) * (Dc ** -0.5)),
            "w_uv": _w((lambda *s: _rng.normal(s) * 0.05)(Dc, H, D) * (Dc ** -0.5)),
            "w_o": _w((lambda *s: _rng.normal(s) * 0.05)(H, D, M) * ((H * D) ** -0.5)),
        }
    _A_in = _A_setup()

    def _B_setup():
        B, S, D, F = 2, 1, 512, 1792
        return {
            "x": _w((lambda *s: _rng.normal(s) * 0.05)(B, S, D)),
            "w1": _w((lambda *s: _rng.normal(s) * 0.05)(D, F) * (D ** -0.5)),
            "b1": _w((lambda *s: _rng.normal(s) * 0.05)(F) * 0.01),
            "w2": _w((lambda *s: _rng.normal(s) * 0.05)(F, D) * (F ** -0.5)),
            "b2": _w((lambda *s: _rng.normal(s) * 0.05)(D) * 0.01),
        }
    _B_in = _B_setup()

    return {
        "A_x": _A_in["x"],
        "A_c_kv": _A_in["c_kv"],
        "A_w_q": _A_in["w_q"],
        "A_w_uk": _A_in["w_uk"],
        "A_w_uv": _A_in["w_uv"],
        "A_w_o": _A_in["w_o"],
        "B_x": _B_in["x"],
        "B_w1": _B_in["w1"],
        "B_b1": _B_in["b1"],
        "B_w2": _B_in["w2"],
        "B_b2": _B_in["b2"],
    }

def reference(A_x, A_c_kv, A_w_q, A_w_uk, A_w_uv, A_w_o, B_x, B_w1, B_b1, B_w2, B_b2):
    def _A_ref(x, c_kv, w_q, w_uk, w_uv, w_o):
        B, Sq, M = x.shape[0], x.shape[1], x.shape[2]
        Sk = c_kv.shape[1]
        H, D = w_q.shape[1], w_q.shape[2]
        q = jnp.einsum("bqm,mhd->bhqd", x, w_q)
        k = jnp.einsum("bkc,chd->bhkd", c_kv, w_uk)
        v = jnp.einsum("bkc,chd->bhkd", c_kv, w_uv)
        scores = jnp.einsum("bhqd,bhkd->bhqk", q, k) * (D ** -0.5)
        off = Sk - Sq
        qi = jnp.arange(Sq)[:, None]
        kj = jnp.arange(Sk)[None, :]
        cmask = kj <= (qi + off)
        scores = jnp.where(cmask[None, None], scores, -1e9)
        p = _softmax(scores, axis=-1)
        ctx = jnp.einsum("bhqk,bhkd->bhqd", p, v)
        return jnp.einsum("bhqd,hdm->bqm", ctx, w_o)

    def _B_ref(x, w1, b1, w2, b2):
        h = jnp.einsum("bsd,df->bsf", x, w1) + b1
        h = _gelu(h)
        return jnp.einsum("bsf,fd->bsd", h, w2) + b2

    x = A_x
    xn = _layernorm(x, axis=-1)
    s = _A_ref(xn, A_c_kv, A_w_q, A_w_uk, A_w_uv, A_w_o)
    g = _silu(_B_ref(xn, B_w1, B_b1, B_w2, B_b2))
    return x + s * g
```

```python
import contextlib
import jax
import jax.numpy as jnp
from jax import lax
import jax.experimental.pallas as pl
import jax.experimental.pallas.tpu as pltpu

F32 = jnp.float32
BF16 = jnp.bfloat16

B, H, SK, D, M, DC, F = 2, 32, 16384, 128, 512, 512, 1792
LOG2E = 1.4426950408889634
NT = (((1,), (1,)), ((), ()))

W_VIEW = (4, 128, H, D)
C_RUNS = 16
C_VIEW = (B * C_RUNS, SK // C_RUNS, DC)
O_VIEW = (4, 8 * D, M)
W1_VIEW = (M // 8 * (F // 128), 8, 128)
BK = 128 * C_RUNS


def _loop(lo, hi, body):
    lax.fori_loop(lo, hi, lambda i, _: body(i), None)


def _rows8(v):
    return jnp.concatenate([v[:, j * 128:(j + 1) * 128] for j in range(M // 128)], axis=0)


def make(Q=26, ramp=(1, 14), t0=(32, 32, 32, 32), t1=(32, 32, 32, 32), nfill=24, fcol=256, fgrp=(16, 64, 16), cuts=(0, 8, 16, 24, 28, 32),
         dma_only=False, TR=False, nmxu=0, same=False, e1=812, delay=0):
    mark = (lambda n: jax.named_scope('@' + n)) if TR else (lambda n: contextlib.nullcontext())
    fill_rows = nfill * 8 * fcol // M
    n0, n1 = sum(t0), sum(t1) + fill_rows
    assert sum(fgrp) == fill_rows and len(t0) == len(t1)
    end5, end7 = (512, 512 - n0 - n1) if same else (512 - n0, 512 - n1)
    assert end5 % 16 == 0 and end7 % 16 == 0
    tail = []
    r0, r1 = ((3, 512 + end7), (3, 512 + end7 + n0)) if same else ((2, 512 + end5), (3, 512 + end7))
    for i in range(len(t0)):
        tail.append((r0[0], r0[1] + sum(t0[:i]), t0[i]))
        tail.append((r1[0], r1[1] + sum(t1[:i]), t1[i]))
    for i in range(len(fgrp)):
        tail.append((r1[0], r1[1] + sum(t1) + sum(fgrp[:i]), fgrp[i]))
    vpu_heads = sorted({a * 8 + r // D for a, lo, n in tail[nmxu:] for r in range(lo, lo + n, 8)})

    def kernel(x_hbm, ckv_hbm, wq_hbm, wuk_hbm, wuv_hbm, wo_hbm, w1_hbm, b1_hbm, w2_hbm, b2_hbm,
               o_hbm,
               x_buf, b1_buf, b2_buf, c_buf, wq_buf, wuk_buf, wuv_buf, wo_buf, w1_buf, w2_buf,
               xs, t8, qa_ref, acc_ref, m_ref, l_ref, e_buf, ctx_ref, mul_ref, gx_ref, o_buf,
               sems):
        def copy(hbm, buf, idx, sem):
            return lambda: pltpu.make_async_copy(hbm.at[idx], buf.at[idx], sem)

        def wait_filled(buf, sem, name='w'):
            with mark(name):
                pltpu.make_async_copy(buf, buf, sem).wait()

        def w_unit(i, k):
            hbm, buf = ((wuv_hbm, wuv_buf), (wuk_hbm, wuk_buf), (wq_hbm, wq_buf))[i // 2]
            return [copy(hbm, buf, (pl.ds(i % 2 * 2, 2), pl.ds(2 * k, 2)), sems.at[0 + (i // 2)])]

        def f1(k):
            return copy(w1_hbm, w1_buf, pl.ds(8 * k, 8), sems.at[0 + (3)])

        def f2(k):
            return copy(w2_hbm, w2_buf, pl.ds(16 * k, 16), sems.at[0 + (4)])

        def c_unit(k, a):
            row = (k & 63) * 16
            row = row if isinstance(k, int) else pl.multiple_of(row, 16)
            return [copy(ckv_hbm, c_buf, (pl.ds((k >> 6) * C_RUNS + a, 2), pl.ds(row, 16)), sems.at[8 + (k >> 3)])]

        units = []
        for k in range(48):
            units += [[f2(k), f2(64 + k)], w_unit(0, k), [f1(k), f1(64 + k)]] + [w_unit(i, k) for i in range(1, 6)]
        for k in range(48, 64, 2):
            units += [[f2(k), f1(k)]] + [w_unit(i, k) for i in range(6)]
            units += [w_unit(0, k + 1), [f2(k + 1), f1(k + 1)]] + [w_unit(i, k + 1) for i in range(1, 6)]
        c0 = len(units) // 2
        units += [c_unit(k, a) for k in range(128) for a in range(0, C_RUNS, 2)]
        o_parts = [[] for _ in cuts[1:]]
        for k in range(32):
            g = sum(k >= c for c in cuts[1:])
            for a, h in ((0, 0), (2, 0), (0, 1), (2, 1)):
                n = 2 if (a, h) != (2, 1) else (16 * k < end5) + (16 * k < end7)
                if n:
                    c = copy(wo_hbm, wo_buf, (pl.ds(a, n), pl.ds(512 * h + 16 * k, 16)), sems.at[24 + (g)])
                    o_parts[g].append(c)
                    units.append([c])
        if len(units) % 2:
            units[-3:] = [units[-3] + units[-1], units[-2]]
        for i, (a, lo, n) in enumerate(tail[:2 * len(t0)]):
            units.append([copy(wo_hbm, wo_buf, (a, pl.ds(lo, n)), sems.at[24 + len(cuts) + (i)])])
        q0, q1 = units[0::2], units[1::2]
        for i, (a, lo, n) in list(enumerate(tail))[2 * len(t0):]:
            q1 += [[copy(wo_hbm, wo_buf, (a, pl.ds(r, 8), pl.ds(c, fcol)), sems.at[24 + len(cuts) + (i)])] for r in range(lo, lo + n, 8) for c in range(0, M, fcol)]
        end = max(len(q0), len(q1) - Q)

        def start(unit, queue):
            for c in unit:
                c().start(priority=queue)

        def issue(lo, hi):
            with mark(f'i{hi}'):
                for i in range(lo, hi):
                    if len(ramp) <= i < len(q0):
                        start(q0[i], 0)
                    if i + Q < len(q1):
                        start(q1[i + Q], 1)

        def issue_c(lo, hi):
            def body(k):
                for u in range(4):
                    start(c_unit(k, 4 * u), 0)
                    start(c_unit(k + (u + Q) // 4, 4 * ((u + Q) % 4) + 2), 1)
            with mark('ic'):
                _loop(lo, hi, body)

        x_copy = pltpu.make_async_copy(x_hbm, x_buf, sems.at[5 + (0)])
        b1_copy = pltpu.make_async_copy(b1_hbm, b1_buf, sems.at[5 + (1)])
        b2_copy = pltpu.make_async_copy(b2_hbm, b2_buf, sems.at[5 + (2)])

        for i in range(Q):
            if i in ramp:
                if delay and ramp.index(i):
                    pl.delay(delay)
                start(q0[ramp.index(i)], 0)
            start(q1[i], 1)
        issue(0, 16)
        for i, c in enumerate((x_copy, b1_copy, b2_copy)):
            c.start()
            issue(16 + i, 17 + i)
        issue(19, 64)

        if dma_only:
            issue(64, c0)
            issue_c(0, 120)
            issue(c0 + 480, end)
            for c in (x_copy, b1_copy, b2_copy):
                c.wait()
            for i, v in enumerate((wuv_buf, wuk_buf, wq_buf, w1_buf, w2_buf)):
                wait_filled(v, sems.at[0 + (i)])
            for i in range(16):
                wait_filled(c_buf.at[pl.ds(0, C_RUNS), pl.ds(0, 128)], sems.at[8 + (i)])
            for p in o_parts:
                for c in p:
                    c().wait()
            for i, (a, lo, n) in enumerate(tail):
                wait_filled(wo_buf.at[a, pl.ds(lo, n)], sems.at[24 + len(cuts) + (i)], f't{i}')
            o_copy = pltpu.make_async_copy(o_buf, o_hbm, sems.at[5 + (0)])
            o_copy.start()
            o_copy.wait()
            return

        x_copy.wait()
        x = x_buf[...].astype(F32)
        xc = x - jnp.mean(x, axis=-1, keepdims=True)
        var = jnp.mean(xc * xc, axis=-1, keepdims=True)
        xn = (xc * lax.rsqrt(var + 1e-5)).astype(BF16)
        xf = xn.astype(F32)
        for b in range(B):
            for j in range(M // 128):
                cols = slice(j * 128, (j + 1) * 128)
                xs[b, cols, :] = jnp.broadcast_to(xf[b:b + 1, cols], (128, 128)).T
        e_buf[...] = (lax.broadcasted_iota(jnp.int32, (128, 1024), 1) // 8
                      == lax.broadcasted_iota(jnp.int32, (128, 1024), 0)).astype(F32).astype(BF16)
        issue(64, c0)
        issue_c(0, 9)

        wait_filled(wq_buf, sems.at[0 + (2)])

        def q_body(i, carry):
            y0, y1 = carry
            for u in range(8):
                m = pl.ds(i * 8 + u, 1)
                w = wq_buf[i >> 4, (i & 15) * 8 + u].astype(F32)
                y0 = y0 + xs[0, m, :] * w
                y1 = y1 + xs[1, m, :] * w
            return y0, y1

        def q_half(h, carry):
            carry = lax.fori_loop(h * 32, h * 32 + 32, q_body, carry)
            issue_c(9 + h * 4, 13 + h * 4)
            return carry

        y0, y1 = lax.fori_loop(0, 2, q_half, (jnp.zeros((H, D), F32), jnp.zeros((H, D), F32)))
        q = jnp.concatenate([y0, y1, jnp.zeros((128 - B * H, D), F32)], axis=0).astype(BF16)

        wait_filled(wuk_buf, sems.at[0 + (1)])
        group = (lax.broadcasted_iota(jnp.int32, (16, 8, 128), 2) % H) // 8

        def qa_body(i):
            for u in range(8):
                w = wuk_buf[i, pl.ds(u * 16, 16)].reshape(16 * H, D)
                r = lax.dot_general(w, q, NT, preferred_element_type=F32).reshape(16, 4, 8, 128)
                v = jnp.where(group == 0, r[:, 0],
                              jnp.where(group == 1, r[:, 1], jnp.where(group == 2, r[:, 2], r[:, 3])))
                t8[pl.ds(pl.multiple_of((i * 8 + u) * 128, 128), 128), :] = v.reshape(128, 128)
            issue_c(17 + i * 3, 20 + i * 3)

        _loop(0, 4, qa_body)
        sub = lax.broadcasted_iota(jnp.int32, (128, 128), 1) % 8
        for j in range(DC // 128):
            t = t8[pl.ds(j * 1024, 128, stride=8), :]
            for s in range(1, 8):
                t = jnp.where(sub == s, t8[pl.ds(j * 1024 + s, 128, stride=8), :], t)
            qa_ref[:, j * 128:(j + 1) * 128] = (t.T[:B * H] * (D ** -0.5 * LOG2E)).astype(BF16)
        issue_c(29, 31)

        wait_filled(w1_buf, sems.at[0 + (3)])
        wait_filled(w2_buf, sems.at[0 + (4)])
        wait_filled(wuv_buf, sems.at[0 + (0)])
        b1_copy.wait()
        b2_copy.wait()
        w1 = w1_buf[...].reshape(M // 8, F // 128, 8, 128)
        w1 = jnp.concatenate([w1[:, j].reshape(M, 128) for j in range(F // 128)], axis=1)
        hid = jnp.dot(xn, w1, preferred_element_type=F32)
        hid = jax.nn.gelu(hid + b1_buf[...].astype(F32).reshape(1, F), approximate=True).astype(BF16)
        z = jnp.dot(hid, w2_buf[...], preferred_element_type=F32)
        z8 = _rows8(z + b2_buf[...].astype(F32).reshape(1, M))
        gx_ref[0] = z8 * jax.nn.sigmoid(z8)
        gx_ref[1] = _rows8(x)

        def issued(i):
            return jnp.maximum(36 + 5 * i, 17 + 8 * i)

        def batch(b):
            hrows = pl.ds(pl.multiple_of(b * H, H), H)
            m_ref[...] = jnp.full((H, 128), -jnp.inf, F32)
            l_ref[...] = jnp.zeros((H, 128), F32)
            acc_ref[...] = jnp.zeros((H, DC), F32)

            def block(g):
                i = b * 8 + g
                pl.when(i < 14)(lambda: issue_c(issued(i - 1) + jnp.where(i == 8, 5, 0), issued(i)))
                pl.when(i == 14)(lambda: issue(c0 + 484, c0 + 516))
                pl.when(i == 15)(lambda: issue(c0 + 516, c0 + 548))
                runs, rows = pl.ds(b * C_RUNS, C_RUNS), pl.ds(pl.multiple_of(g * 128, 128), 128)
                wait_filled(c_buf.at[runs, rows], sems.at[8 + (i)], 'c')
                c = c_buf[runs, rows].reshape(BK, DC)
                sc = lax.dot_general(qa_ref[hrows, :], c, NT, preferred_element_type=F32)
                m_prev = m_ref[...]
                m_new = jnp.maximum(m_prev, jnp.max(sc, axis=1, keepdims=True))
                p = jnp.exp2(sc - m_new[:, :1])
                alpha = jnp.exp2(m_prev - m_new)
                l_ref[...] = alpha * l_ref[...] + jnp.sum(p, axis=1, keepdims=True)
                m_ref[...] = m_new
                pv = jnp.dot(p.astype(BF16), c, preferred_element_type=F32)
                acc_ref[...] = acc_ref[...] * alpha[:, :1] + pv

            _loop(0, 8, block)
            pl.when(b == 0)(lambda: issue_c(73, 78))
            pl.when(b == 1)(lambda: issue(c0 + 548, e1))
            pc = (acc_ref[...] / l_ref[...][:, :1]).astype(BF16)
            diag = (lax.broadcasted_iota(jnp.int32, (4 * H, 1024), 1) % 8
                    == lax.broadcasted_iota(jnp.int32, (4 * H, 1024), 0) % 8)
            pc4 = jnp.concatenate([pc[:, j * 128:(j + 1) * 128] for j in range(4)], axis=0)
            rep = jnp.where(diag, jnp.dot(pc4, e_buf[...], preferred_element_type=F32), 0.0)
            ctx = jnp.concatenate([
                jnp.dot(jnp.concatenate([rep[j * H + g:j * H + g + 8] for j in range(4)], axis=1).astype(BF16),
                        wuv_buf[:, :, g:g + 8].reshape(DC * 8, D), preferred_element_type=F32)
                for g in range(0, H, 8)], axis=0)
            ctx_ref[hrows] = ctx
            cb = ctx.astype(BF16).astype(F32)
            for k, h in enumerate(vpu_heads):
                mul_ref[b, k * D:(k + 1) * D] = jnp.broadcast_to(cb[h:h + 1], (128, 128)).T

        _loop(0, B, batch)
        issue(e1, end)

        def lhs_of(spans):
            return jnp.concatenate([ctx_ref[pl.ds(a * 8 + lo // D, B, stride=H), :][:, lo % D:lo % D + n]
                                    for a, lo, n in spans], axis=1).astype(BF16)

        def project(spans, lhs):
            rhs = jnp.concatenate([wo_buf[a, lo:lo + n] for a, lo, n in spans], axis=0)
            return jnp.dot(lhs, rhs, preferred_element_type=F32)

        groups = []
        for lo, hi in zip(cuts, cuts[1:]):
            sp = [(a, 512 * h + r, min(16 * hi, stop, r // D * D + D) - r)
                  for a in range(4) for h in range(2) for stop in [{2: end5, 3: end7}.get(a, 512) if h else 512]
                  for r in [16 * lo] + list(range(16 * lo // D * D + D, 16 * hi, D)) if r < stop]
            groups.append(sp)
        lhs = [lhs_of(sp) for sp in groups]
        tl = lhs_of(tail[:nmxu]) if nmxu else None
        s = jnp.zeros((B, M), F32)
        for g, sp in enumerate(groups):
            with mark(f'o{g}'):
                for a, lo, n in sp:
                    v = wo_buf.at[a, pl.ds(lo, n)]
                    pltpu.make_async_copy(v, v, sems.at[24 + (g)]).wait()
            s = s + project(sp, lhs[g])
        for i, (a, lo, n) in enumerate(tail[:nmxu]):
            wait_filled(wo_buf.at[a, pl.ds(lo, n)], sems.at[24 + len(cuts) + (i)], f't{i}')
        if nmxu:
            s = s + project(tail[:nmxu], tl)
        g8 = gx_ref[0]
        base8 = gx_ref[1] + _rows8(s) * g8

        part = [[None] * (M // 128) for _ in range(B)]
        for i, (a, lo, n) in list(enumerate(tail))[nmxu:]:
            wait_filled(wo_buf.at[a, pl.ds(lo, n)], sems.at[24 + len(cuts) + (i)], f't{i}')
            for r in range(lo, lo + n, 8):
                w = wo_buf[a, r:r + 8].astype(F32)
                at = vpu_heads.index(a * 8 + r // D) * D + r % D
                for b in range(B):
                    mul = mul_ref[b, at:at + 8, :]
                    for j in range(M // 128):
                        t = w[:, j * 128:(j + 1) * 128] * mul
                        part[b][j] = t if part[b][j] is None else part[b][j] + t

        sl = lax.broadcasted_iota(jnp.int32, (8, 128), 0)

        def merge(lo, hi, k):
            m = (sl & k) != 0
            if k == 4:
                return jnp.where(m, hi, lo) + pltpu.roll(jnp.where(m, lo, hi), 4, 0)
            return jnp.where(m, hi, lo) + jnp.where(m, pltpu.roll(hi, k, 0), pltpu.roll(lo, 8 - k, 0))

        r4 = [[merge(part[b][j], part[b][j + 2], 4) for j in range(2)] for b in range(B)]
        r2 = [merge(r4[b][0], r4[b][1], 2) for b in range(B)]
        o_buf[...] = (base8 + g8 * merge(r2[0], r2[1], 1)).astype(BF16)
        o_copy = pltpu.make_async_copy(o_buf, o_hbm, sems.at[5 + (0)])
        o_copy.start()
        o_copy.wait()

    def fn(A_x, A_c_kv, A_w_q, A_w_uk, A_w_uv, A_w_o, B_x, B_w1, B_b1, B_w2, B_b2):
        hbm = pl.BlockSpec(memory_space=pltpu.HBM)
        dma_sems = pltpu.SemaphoreType.DMA
        out = pl.pallas_call(
            kernel,
            out_shape=jax.ShapeDtypeStruct((8, 128), BF16),
            in_specs=[hbm] * 10,
            out_specs=hbm,
            scratch_shapes=[
                pltpu.VMEM((B, M), BF16), pltpu.VMEM((F,), BF16), pltpu.VMEM((M,), BF16),
                pltpu.VMEM(C_VIEW, BF16), pltpu.VMEM(W_VIEW, BF16), pltpu.VMEM(W_VIEW, BF16),
                pltpu.VMEM(W_VIEW, BF16), pltpu.VMEM(O_VIEW, BF16),
                pltpu.VMEM(W1_VIEW, BF16), pltpu.VMEM((F, M), BF16),
                pltpu.VMEM((B, M, 128), F32),
                pltpu.VMEM((DC * 8 + 8, 128), F32),
                pltpu.VMEM((B * H, DC), BF16), pltpu.VMEM((H, DC), F32),
                pltpu.VMEM((H, 128), F32), pltpu.VMEM((H, 128), F32),
                pltpu.VMEM((128, 1024), BF16),
                pltpu.VMEM((3 * H, D), F32), pltpu.VMEM((B, len(vpu_heads) * D, 128), F32),
                pltpu.VMEM((2, 8, 128), F32), pltpu.VMEM((8, 128), BF16),
                dma_sems((24 + len(cuts) + len(tail),)),
            ],
            compiler_params=pltpu.CompilerParams(
                vmem_limit_bytes=100 * 1024 * 1024, disable_semaphore_checks=True, disable_bounds_checks=True),
        )(A_x.reshape(B, M), A_c_kv.reshape(C_VIEW), A_w_q.reshape(W_VIEW), A_w_uk.reshape(W_VIEW),
          A_w_uv.reshape(W_VIEW), A_w_o.reshape(O_VIEW),
          B_w1.reshape(M // 8, 8, F // 128, 128).transpose(0, 2, 1, 3).reshape(W1_VIEW), B_b1, B_w2, B_b2)
        return out.reshape(M // 128, B, 128).transpose(1, 0, 2).reshape(B, 1, M)
    return fn


_impl = make()


@jax.jit
def pallas_recurrent_scan__compressed_kv_cla__dense_activation_gelu__decode_kernel(
    A_x, A_c_kv, A_w_q, A_w_uk, A_w_uv, A_w_o, B_x, B_w1, B_b1, B_w2, B_b2,
):
    return _impl(A_x, A_c_kv, A_w_q, A_w_uk, A_w_uv, A_w_o, B_x, B_w1, B_b1, B_w2, B_b2)
```

```python
import contextlib
import jax
import jax.numpy as jnp
from jax import lax
import jax.experimental.pallas as pl
import jax.experimental.pallas.tpu as pltpu

F32 = jnp.float32
BF16 = jnp.bfloat16

B, H, SK, D, M, DC, F = 2, 32, 16384, 128, 512, 512, 1792
LOG2E = 1.4426950408889634
NT = (((1,), (1,)), ((), ()))

W_VIEW = (4, 128, H, D)
C_RUNS = 16
C_VIEW = (B * C_RUNS, SK // C_RUNS, DC)
O_VIEW = (4, 4096, 128)
W1_VIEW = (M // 8 * (F // 128), 8, 128)
BK = 128 * C_RUNS


def _loop(lo, hi, body):
    lax.fori_loop(lo, hi, lambda i, _: body(i), None)


def _rows8(v):
    return jnp.concatenate([v[:, j * 128:(j + 1) * 128] for j in range(M // 128)], axis=0)


def make(Q=26, ramp=(2, 16), t0=(32, 32, 32, 32), t1=(8, 8, 8, 8), nfill=24, fgrp=(8, 6, 4, 4, 2), cuts=(0, 8, 16, 20, 27), e1=12, e2=12,
         dma_only=False, TR=False, two=False, small=40, tgrp=2, pos=(540, 552, 564, 572, 580, 596), nfast=4, notail=False, noatt=False, perm=(0, 4, 8, 1, 5, 9, 2, 6, 10, 3, 7, 11), defer=True, hv=0, pre=True):
    mark = (lambda n: jax.named_scope('@' + n)) if TR else (lambda n: contextlib.nullcontext())
    nt = sum(t0) + sum(t1) + 4 * nfill
    assert sum(fgrp) == nfill and nt % 16 == 0 and nfill % 2 == 0
    end7 = 512 - nt
    tail, row = [], 4096 - nt
    for n in [n for p in zip(t0, t1) for n in p]:
        tail.append((row, n, 0, M))
        row += n
    fill = [(r, 8, c, 256) for r in range(row, 4096, 8) for c in (0, 256)]
    if perm:
        fill = [fill[2 * i + u] for i in perm for u in range(2)]
    fast = [f[0] for f in fill[-sum(fgrp[-nfast:])::2]]
    waits = [tail[i:i + tgrp] for i in range(0, len(tail), tgrp)] + [fill[sum(fgrp[:i]):sum(fgrp[:i + 1])] for i in range(len(fgrp))]
    rw = [(k, p) for k in range(cuts[-1], 32) for p in (((0, 1, 2, 3), (4, 5, 6, 7)) if k >= 32 - hv else (tuple(range(8)),))]
    nv = len(rw)
    waits = [[(512 * r + 16 * k, 16, 0, M) for r in p if 512 * r + 16 * k < 4096 - nt] for k, p in rw] + waits
    vpu_heads = sorted({r // D for w in waits for lo, n, _, _ in w for r in range(lo, lo + n, 8)})
    pv = (lambda v: (v[0] // 4, 2, 2) + v[1:]) if two else (lambda v: v)

    def kernel(x_hbm, ckv_hbm, wq_hbm, wuk_hbm, wuv_hbm, wo_hbm, w1_hbm, b1_hbm, w2_hbm, b2_hbm,
               o_hbm,
               c_buf, wq_buf, wuk_buf, wuv_buf, wo_buf, w1_buf, w2_buf,
               xs, t8, qa_ref, acc_ref, m_ref, l_ref, e_buf, ctx_ref, mul_ref, gm_ref, o_buf, b1_buf, x_buf, b2_buf,
               sems):
        def copy(hbm, buf, idx, sem):
            return lambda: pltpu.make_async_copy(hbm.at[idx], buf.at[idx], sem)

        def wait_filled(buf, sem, name='w'):
            with mark(name):
                pltpu.make_async_copy(buf, buf, sem).wait()

        def pair(hbm, buf, a, rows, sem):
            return [copy(hbm, buf, (a // 4, slice(None), a // 2 % 2, rows) if two else (pl.ds(a, 2), rows), sem)]

        def w_unit(i, k):
            hbm, buf = ((wuv_hbm, wuv_buf), (wuk_hbm, wuk_buf), (wq_hbm, wq_buf))[i // 2]
            return pair(hbm, buf, i % 2 * 2, pl.ds(2 * k, 2), sems.at[i // 2])

        def ffn(k, *rows):
            return [copy(w2_hbm, w2_buf, pl.ds(16 * f, 16), sems.at[4]) if f < 112 else copy(w1_hbm, w1_buf, pl.ds(8 * (f - 112), 8), sems.at[3])
                    for f in [32 * r + k for r in rows]]

        def c_unit(k, a):
            row = (k & 63) * 16
            row = row if isinstance(k, int) else pl.multiple_of(row, 16)
            b = k >> 6
            idx = (b * 4 + a // 4, slice(None), a // 2 % 2) if two else (pl.ds(b * C_RUNS + a, 2),)
            return [copy(ckv_hbm, c_buf, idx + (pl.ds(row, 16),), sems.at[8 + (k >> 3)])]

        units = []

        def add(pairs, singles):
            while pairs or singles:
                units.append(singles.pop(0) if singles and len(units) % 2 == 0 else pairs.pop(0))

        for k in range(64):
            add([w_unit(i, k) for i in range(6)],
                ([ffn(k, 1) if k < 32 else ffn(k, -1, 1)] if k % 32 >= 32 - e2 else []) + ([ffn(k, 3, 5)] if k % 32 >= 32 - e1 else []))
        assert len(units) % 2 == 0
        c0 = len(units) // 2
        units += [c_unit(k, a) for k in range(128) for a in range(0, C_RUNS, 2)]
        for k in range(32):
            g = lambda a: sum(k >= c for c in cuts[1:]) if k < cuts[-1] else len(cuts) + [kk == k and 2 * a in p for kk, p in rw].index(True)
            p8, p12, p7, p11 = [[copy(wo_hbm, wo_buf, (pl.ds(a, 2 - ((a, h) == (2, 1) and 16 * k >= end7)), pl.ds(2048 * h + 64 * k, 64)), sems.at[24 + g(a)])]
                                for h in (1, 0) for a in (0, 2)]
            if k < 32 - e1:
                add([p8, p12, p7, p11], [ffn(k, 0, 2), ffn(k, 4, 6), ffn(k, 1, 3), ffn(k, 5)])
            elif k < 32 - e2:
                add([p8, p7, p11], [ffn(k, 0, 2), p12 + ffn(k, 1)])
            else:
                add([p8, p7, p12, p11], [])
        assert len(units) % 2 == 0
        last = [[copy(wo_hbm, wo_buf, (3, pl.ds(r % 1024 * 4 + c // 16, n * m // 128)), sems.at[24 + len(cuts) + i])] for i, w in list(enumerate(waits))[nv:] for r, n, c, m in w]
        units += last[:len(tail)]
        q0, q1 = units[0::2], units[1::2] + last[len(tail):]
        end = max(len(q0), len(q1) - Q)

        groups = []
        for lo, hi in zip(cuts, cuts[1:]):
            groups.append([(a, 512 * h + r, min(16 * hi, stop, r // D * D + D) - r)
                           for a in range(4) for h in range(2) for stop in [end7 if (a, h) == (3, 1) else 512]
                           for r in [16 * lo] + list(range(16 * lo // D * D + D, 16 * hi, D)) if r < stop])

        def wait_group(g):
            with mark(f'o{g}'):
                for a, lo, n in groups[g]:
                    v = wo_buf.at[a, pl.ds(4 * lo, 4 * n)]
                    pltpu.make_async_copy(v, v, sems.at[24 + g]).wait()

        def wait_last(i):
            with mark(f't{i}'):
                for r, n, c, m in waits[i]:
                    v = wo_buf.at[r // 1024, pl.ds(r % 1024 * 4 + c // 16, n * m // 128)]
                    pltpu.make_async_copy(v, v, sems.at[24 + len(cuts) + i]).wait()

        def start(unit, queue):
            for c in unit:
                c().start(priority=queue)

        def issue(lo, hi):
            with mark(f'i{hi}'):
                for i in range(lo, hi):
                    if len(ramp) <= i < len(q0):
                        start(q0[i], 0)
                    if i + Q < len(q1):
                        start(q1[i + Q], 1)

        def issue_c(lo, hi):
            def body(k):
                for u in range(4):
                    start(c_unit(k, 4 * u), 0)
                    start(c_unit(k + (u + Q) // 4, 4 * ((u + Q) % 4) + 2), 1)
            with mark('ic'):
                _loop(lo, hi, body)

        x_copy = pltpu.make_async_copy(x_hbm, x_buf, sems.at[5 + (0)])
        b1_copy = pltpu.make_async_copy(b1_hbm, b1_buf, sems.at[5 + (1)])
        b2_copy = pltpu.make_async_copy(b2_hbm, b2_buf, sems.at[5 + (2)])

        for i in range(Q):
            if i in ramp:
                start(q0[ramp.index(i)], 0)
            start(q1[i], 1)
        issue(0, small)
        for i, c in enumerate((x_copy, b1_copy, b2_copy)):
            c.start()
            issue(small + i, small + 1 + i)
        issue(small + 3, 64)

        if dma_only:
            issue(64, c0)
            issue_c(0, 120)
            issue(c0 + 480, end)
            for c in (x_copy, b1_copy, b2_copy):
                c.wait()
            for i, v in enumerate((wuv_buf, wuk_buf, wq_buf, w1_buf, w2_buf)):
                wait_filled(v, sems.at[0 + (i)])
            for i in range(16):
                wait_filled(c_buf.at[pl.ds(0, 4), :, :, pl.ds(0, 128)] if two else c_buf.at[pl.ds(0, C_RUNS), pl.ds(0, 128)], sems.at[8 + i])
            for g in range(len(groups)):
                wait_group(g)
            for i in range(len(waits)):
                wait_last(i)
            o_copy = pltpu.make_async_copy(o_buf, o_hbm, sems.at[5 + (0)])
            o_copy.start()
            o_copy.wait()
            return

        x_copy.wait()
        x = x_buf[...].astype(F32)
        xc = x - jnp.mean(x, axis=-1, keepdims=True)
        var = jnp.mean(xc * xc, axis=-1, keepdims=True)
        xn = (xc * lax.rsqrt(var + 1e-5)).astype(BF16)
        xf = xn.astype(F32)
        for b in range(B):
            for j in range(M // 128):
                cols = slice(j * 128, (j + 1) * 128)
                xs[b, cols, :] = jnp.broadcast_to(xf[b:b + 1, cols], (128, 128)).T
        e_buf[...] = (lax.broadcasted_iota(jnp.int32, (128, 1024), 1) // 8
                      == lax.broadcasted_iota(jnp.int32, (128, 1024), 0)).astype(F32).astype(BF16)
        issue(64, c0)
        issue_c(0, 9)

        wait_filled(wq_buf, sems.at[0 + (2)])

        def q_body(i, carry):
            y0, y1 = carry
            for u in range(8):
                m = pl.ds(i * 8 + u, 1)
                w = wq_buf[i >> 4, (i & 15) * 8 + u].astype(F32)
                y0 = y0 + xs[0, m, :] * w
                y1 = y1 + xs[1, m, :] * w
            return y0, y1

        def q_half(h, carry):
            carry = lax.fori_loop(h * 32, h * 32 + 32, q_body, carry)
            issue_c(9 + h * 4, 13 + h * 4)
            return carry

        y0, y1 = lax.fori_loop(0, 2, q_half, (jnp.zeros((H, D), F32), jnp.zeros((H, D), F32)))
        q = jnp.concatenate([y0, y1, jnp.zeros((128 - B * H, D), F32)], axis=0).astype(BF16)

        wait_filled(wuk_buf, sems.at[0 + (1)])
        group = (lax.broadcasted_iota(jnp.int32, (16, 8, 128), 2) % H) // 8

        def qa_body(i):
            for u in range(8):
                w = wuk_buf[i, pl.ds(u * 16, 16)].reshape(16 * H, D)
                r = lax.dot_general(w, q, NT, preferred_element_type=F32).reshape(16, 4, 8, 128)
                v = jnp.where(group == 0, r[:, 0],
                              jnp.where(group == 1, r[:, 1], jnp.where(group == 2, r[:, 2], r[:, 3])))
                t8[pl.ds(pl.multiple_of((i * 8 + u) * 128, 128), 128), :] = v.reshape(128, 128)
            issue_c(17 + i * 3, 20 + i * 3)

        _loop(0, 4, qa_body)
        sub = lax.broadcasted_iota(jnp.int32, (128, 128), 1) % 8
        for j in range(DC // 128):
            t = t8[pl.ds(j * 1024, 128, stride=8), :]
            for s in range(1, 8):
                t = jnp.where(sub == s, t8[pl.ds(j * 1024 + s, 128, stride=8), :], t)
            qa_ref[:, j * 128:(j + 1) * 128] = (t.T[:B * H] * (D ** -0.5 * LOG2E)).astype(BF16)
        pass

        wait_filled(wuv_buf, sems.at[0])

        def issued(i):
            return jnp.maximum(34 + 5 * i, 17 + 8 * i)

        def batch(b):
            hrows = pl.ds(pl.multiple_of(b * H, H), H)
            m_ref[...] = jnp.full((H, 128), -jnp.inf, F32)
            l_ref[...] = jnp.zeros((H, 128), F32)
            acc_ref[...] = jnp.zeros((H, DC), F32)

            def block(g):
                i = b * 8 + g
                pl.when(i < 14)(lambda: issue_c(issued(i - 1) + jnp.where(i == 8, 7, 0), issued(i)))
                pl.when(i == 14)(lambda: issue(c0 + 484, c0 + 516))
                pl.when(i == 15)(lambda: issue(c0 + 526, c0 + pos[0]))
                runs, rows = pl.ds(b * C_RUNS, C_RUNS), pl.ds(pl.multiple_of(g * 128, 128), 128)
                wait_filled(c_buf.at[runs, rows], sems.at[8 + (i)], 'c')
                if noatt:
                    pl.delay(noatt)
                    pl.when(i == 14)(lambda: issue(c0 + 516, c0 + 526))
                    pl.when(i == 15)(lambda: issue(c0 + pos[0], c0 + pos[1]))
                    return
                c = c_buf[runs, rows].reshape(BK, DC)
                sc = lax.dot_general(qa_ref[hrows, :], c, NT, preferred_element_type=F32)
                m_prev = m_ref[...]
                m_new = jnp.maximum(m_prev, jnp.max(sc, axis=1, keepdims=True))
                p = jnp.exp2(sc - m_new[:, :1])
                alpha = jnp.exp2(m_prev - m_new)
                l_ref[...] = alpha * l_ref[...] + jnp.sum(p, axis=1, keepdims=True)
                m_ref[...] = m_new
                p = p.astype(BF16)
                pl.when(i == 14)(lambda: issue(c0 + 516, c0 + 526))
                pl.when(i == 15)(lambda: issue(c0 + pos[0], c0 + pos[1]))
                pv = jnp.dot(p, c_buf[runs, rows].reshape(BK, DC), preferred_element_type=F32)
                acc_ref[...] = acc_ref[...] * alpha[:, :1] + pv

            _loop(0, 8, block)
            pl.when(b == 0)(lambda: issue_c(73, 78))
            pl.when(b == 1)(lambda: issue(c0 + pos[1], c0 + pos[2]))
            pc = (acc_ref[...] / l_ref[...][:, :1]).astype(BF16)
            diag = (lax.broadcasted_iota(jnp.int32, (4 * H, 1024), 1) % 8
                    == lax.broadcasted_iota(jnp.int32, (4 * H, 1024), 0) % 8)
            pc4 = jnp.concatenate([pc[:, j * 128:(j + 1) * 128] for j in range(4)], axis=0)
            rep = jnp.where(diag, jnp.dot(pc4, e_buf[...], preferred_element_type=F32), 0.0)
            ctx = []
            for g in range(0, H, 8):
                if g == 16:
                    pl.when(b == 0)(lambda: issue_c(78, 80))
                    pl.when(b == 1)(lambda: issue(c0 + pos[2], c0 + pos[3]))
                ctx.append(jnp.dot(jnp.concatenate([rep[j * H + g:j * H + g + 8] for j in range(4)], axis=1).astype(BF16),
                                   wuv_buf[:, :, g:g + 8].reshape(DC * 8, D), preferred_element_type=F32))
            ctx = jnp.concatenate(ctx, axis=0)
            ctx_ref[hrows] = ctx
            cb = ctx.astype(BF16).astype(F32)
            for k, h in enumerate(vpu_heads):
                mul_ref[b, k * D:(k + 1) * D] = jnp.broadcast_to(cb[h:h + 1], (128, 128)).T

        _loop(0, B, batch)
        issue(c0 + pos[3], c0 + pos[4])

        def lhs_of(spans):
            return jnp.concatenate([ctx_ref[pl.ds(a * 8 + lo // D, B, stride=H), :][:, lo % D:lo % D + n]
                                    for a, lo, n in spans], axis=1).astype(BF16)

        def project(spans, lhs):
            w = jnp.concatenate([wo_buf[a, pl.ds(4 * lo, 4 * n)].reshape(n // 8, 4, 8, 128) for a, lo, n in spans], axis=0)
            rhs = jnp.concatenate([w[:, j].reshape(-1, 128) for j in range(4)], axis=1)
            return jnp.dot(lhs, rhs, preferred_element_type=F32)

        lhs = [lhs_of(sp) for sp in groups]
        sl = lax.broadcasted_iota(jnp.int32, (8, 128), 0)
        odd = (sl & 1) == 1

        def mul_rows(b, r, n):
            return mul_ref[b, pl.ds(vpu_heads.index(r // D) * D + r % D, n), :]

        s = jnp.zeros((B, M), F32)
        for g, sp in enumerate(groups):
            if g == 1:
                issue(c0 + pos[4], c0 + pos[5])
            if g == 2:
                issue(c0 + pos[5], end)
            wait_group(g)
            s = s + project(sp, lhs[g])
            if cuts[g] < 32 - e1 <= cuts[g + 1]:
                wait_filled(w1_buf, sems.at[3], 'w1')
                b1_copy.wait()
                w1 = w1_buf[...].reshape(M // 8, F // 128, 8, 128)
                w1 = jnp.concatenate([w1[:, j].reshape(M, 128) for j in range(F // 128)], axis=1)
                hid = jnp.dot(xn, w1, preferred_element_type=F32)
                hid = jax.nn.gelu(hid + b1_buf[...].astype(F32).reshape(1, F), approximate=True).astype(BF16)
            if cuts[g] < 32 - e2 <= cuts[g + 1]:
                wait_filled(w2_buf, sems.at[4], 'w2')
                b2_copy.wait()
                z = jnp.dot(hid, w2_buf[...], preferred_element_type=F32)
                z8 = _rows8(z + b2_buf[...].astype(F32).reshape(1, M))
                g8 = z8 * jax.nn.sigmoid(z8)
                gb = [jnp.where(odd, pltpu.roll(g8, 1, 0), g8), jnp.where(odd, g8, pltpu.roll(g8, 7, 0))]
                for b in range(B):
                    for r in fast:
                        for u in range(4):
                            gm_ref[b, 4 * fast.index(r) + u] = jnp.where(odd, mul_rows(b, r + 4 + u, 1), mul_rows(b, r + u, 1)) * gb[b]
        base8 = _rows8(x) + _rows8(s) * g8

        def merge(lo, hi, k):
            m = (sl & k) != 0
            if k == 4:
                return jnp.where(m, hi, lo) + pltpu.roll(jnp.where(m, lo, hi), 4, 0)
            return jnp.where(m, hi, lo) + jnp.where(m, pltpu.roll(hi, k, 0), pltpu.roll(lo, 8 - k, 0))

        own = [jnp.where(odd == (b == 1), base8, 0.0) for b in range(B)]
        part = [[None] * (M // 128) for _ in range(B)]
        if notail:
            o_buf[...] = base8.astype(BF16)
            for i in range(len(waits)):
                wait_last(i)
        else:
            def add_part(terms):
                for b, j, t in terms:
                    part[b][j] = t if part[b][j] is None else part[b][j] + t

            terms = []
            for i in range(len(waits) - nfast):
                if not defer:
                    add_part(terms)
                    terms = []
                wait_last(i)
                for lo, n, c, m in waits[i]:
                    for r in range(lo, lo + n, 8):
                        w = wo_buf[r // 1024, pl.ds(r % 1024 * 4 + c // 16, m // 16)].astype(F32)
                        add_part(terms)
                        terms = [(b, j, w[8 * j - c // 16:8 * j - c // 16 + 8] * mul_rows(b, r, 8)) for b in range(B) for j in range(c // 128, (c + m) // 128)]

            def fold():
                add_part(terms)
                r4 = [[merge(part[b][j], part[b][j + 2], 4) for j in range(2)] for b in range(B)]
                return [merge(r4[b][0], r4[b][1], 2) * gb[b] + own[b] for b in range(B)]

            acc = None if defer else fold()
            words = wo_buf.bitcast(jnp.uint32)
            pend = []
            for i in range(len(waits) - nfast, len(waits)):
                r = waits[i][0][0]
                gm = {r: gm_ref[:, pl.ds(4 * fast.index(r), 4)]} if pre else {}
                wait_last(i)
                for r, _, c, _ in waits[i][::2]:
                    w = []
                    for u in range(2):
                        v = words[3, pl.ds(r % 1024 * 2 + u, 8, stride=2), :]
                        w += [lax.bitcast_convert_type(v << 16, F32), lax.bitcast_convert_type(v & jnp.uint32(0xFFFF0000), F32)]
                    acc = acc or fold()
                    for b, t in pend:
                        acc[b] = acc[b] + ((t[0] + t[1]) + (t[2] + t[3]))
                    f = gm[r] if r in gm else gm_ref[:, pl.ds(4 * fast.index(r), 4)]
                    pend = [(b, [w[u] * f[b, u] for u in range(4)]) for b in range(B)]
                if not defer or i == len(waits) - 1:
                    for b, t in pend:
                        acc[b] = ((acc[b] + t[0]) + t[1]) + (t[2] + t[3])
                    pend = []
            out = jnp.where(odd, acc[1] + pltpu.roll(acc[1], 1, 0), acc[0] + pltpu.roll(acc[0], 7, 0))
            o_buf[...] = out.astype(BF16)
        o_copy = pltpu.make_async_copy(o_buf, o_hbm, sems.at[5 + (0)])
        o_copy.start()
        o_copy.wait()

    def fn(A_x, A_c_kv, A_w_q, A_w_uk, A_w_uv, A_w_o, B_x, B_w1, B_b1, B_w2, B_b2):
        hbm = pl.BlockSpec(memory_space=pltpu.HBM)
        dma_sems = pltpu.SemaphoreType.DMA
        out = pl.pallas_call(
            kernel,
            out_shape=jax.ShapeDtypeStruct((8, 128), BF16),
            in_specs=[hbm] * 10,
            out_specs=hbm,
            scratch_shapes=[
                pltpu.VMEM(pv(C_VIEW), BF16), pltpu.VMEM(pv(W_VIEW), BF16), pltpu.VMEM(pv(W_VIEW), BF16),
                pltpu.VMEM(pv(W_VIEW), BF16), pltpu.VMEM((4, 4096 + 16, 128), BF16),
                pltpu.VMEM(W1_VIEW, BF16), pltpu.VMEM((F, M), BF16),
                pltpu.VMEM((B, M, 128), F32),
                pltpu.VMEM((DC * 8 + 8, 128), F32),
                pltpu.VMEM((B * H, DC), BF16), pltpu.VMEM((H, DC), F32),
                pltpu.VMEM((H, 128), F32), pltpu.VMEM((H, 128), F32),
                pltpu.VMEM((128, 1024), BF16),
                pltpu.VMEM((3 * H, D), F32), pltpu.VMEM((B, len(vpu_heads) * D, 128), F32),
                pltpu.VMEM((B, 4 * len(fast), 8, 128), F32), pltpu.VMEM((8, 128), BF16),
                pltpu.VMEM((F,), BF16), pltpu.VMEM((B, M), BF16), pltpu.VMEM((M,), BF16),
                dma_sems((24 + len(cuts) + len(waits),)),
            ],
            compiler_params=pltpu.CompilerParams(
                vmem_limit_bytes=100 * 1024 * 1024, disable_semaphore_checks=True, disable_bounds_checks=True),
        )(A_x.reshape(B, M), A_c_kv.reshape(pv(C_VIEW)), A_w_q.reshape(pv(W_VIEW)), A_w_uk.reshape(pv(W_VIEW)),
          A_w_uv.reshape(pv(W_VIEW)), A_w_o.reshape(512, 8, 4, 128).transpose(0, 2, 1, 3).reshape(O_VIEW),
          B_w1.reshape(M // 8, 8, F // 128, 128).transpose(0, 2, 1, 3).reshape(W1_VIEW), B_b1, B_w2, B_b2)
        return out.reshape(M // 128, B, 128).transpose(1, 0, 2).reshape(B, 1, M)
    return fn


_impl = make(pre=False)


@jax.jit
def pallas_recurrent_scan__compressed_kv_cla__dense_activation_gelu__decode_kernel(
    A_x, A_c_kv, A_w_q, A_w_uk, A_w_uv, A_w_o, B_x, B_w1, B_b1, B_w2, B_b2,
):
    return _impl(A_x, A_c_kv, A_w_q, A_w_uk, A_w_uv, A_w_o, B_x, B_w1, B_b1, B_w2, B_b2)
```

```python
import jax
import jax.numpy as jnp
from jax import lax
import jax.experimental.pallas as pl
import jax.experimental.pallas.tpu as pltpu

F32 = jnp.float32
BF16 = jnp.bfloat16

B, H, SK, D, M, DC, F = 2, 32, 16384, 128, 512, 512, 1792
LOG2E = 1.4426950408889634
NT = (((1,), (1,)), ((), ()))

LEAD = 26
W_VIEW = (4, 128, H, D)
C_RUNS = 16
C_VIEW = (B * C_RUNS, SK // C_RUNS, DC)
O_VIEW = (4, 8 * D, M)
W1_VIEW = (M // 8 * F // 128, 8, 128)
BLOCKS = 8
LATE = 20
MXU_CUTS = (0, 8, 16, LATE, 27)
END_UNITS = (24, 8) * 3
END_TINY = ((0, 4, 8, 1), (5, 9, 2), (6, 10), (3, 7), (11,))
VPU_HEADS = tuple(range(3, H - 4, 4)) + tuple(range(H - 4 + LATE // 8, H))
SEM_W, SEM_FFN, SEM_SMALL, SEM_C = 0, 3, 5, 9
SEM_O = SEM_C + B * BLOCKS
O_PARTS = len(MXU_CUTS) - 1 + 32 - MXU_CUTS[-1] + len(END_UNITS) // 2 + len(END_TINY)


def _loop(lo, hi, body):
    lax.fori_loop(lo, hi, lambda i, _: body(i), None)


def _rows8(v):
    return jnp.concatenate([v[:, j * 128:(j + 1) * 128] for j in range(M // 128)], axis=0)


def _kernel(x_hbm, ckv_hbm, wq_hbm, wuk_hbm, wuv_hbm, wo_hbm, w1_hbm, b1_hbm, w2_hbm, b2_hbm,
            o_hbm,
            c_buf, wq_buf, wuk_buf, wuv_buf, wo_buf, w1_buf, w2_buf,
            xs, t8, qa_ref, acc_ref, m_ref, l_ref, e_buf, ctx_ref, mul_ref, o_buf, b1_buf, x_buf, b2_buf,
            sems):
    def copy(hbm, buf, idx, sem):
        return pltpu.make_async_copy(hbm.at[idx], buf.at[idx], sems.at[sem])

    def wait_filled(buf, sem):
        pltpu.make_async_copy(buf, buf, sems.at[sem]).wait()

    def ffn_unit(k, *halves):
        n = F // 16
        return [(w2_hbm, w2_buf, pl.ds(16 * i, 16), SEM_FFN + 1) if i < n else
                (w1_hbm, w1_buf, pl.ds(8 * (i - n), 8), SEM_FFN)
                for i in [32 * h + k for h in halves] if i >= 0]

    def c_unit(k, a):
        row = (k & 63) * 16
        row = row if isinstance(k, int) else pl.multiple_of(row, 16)
        return [(ckv_hbm, c_buf, (pl.ds((k >> 6) * C_RUNS + a, 2), pl.ds(row, 16)), SEM_C + (k >> 3))]

    o_parts = [[] for _ in range(O_PARTS)]

    def o_unit(part, a, runs, row, rows, col=0, cols=M):
        piece = (wo_hbm, wo_buf, (pl.ds(a, runs), pl.ds(row, rows), pl.ds(col, cols)), SEM_O + part)
        o_parts[part].append(piece)
        return [piece]

    units = []
    for k in range(64):
        w = [[(hbm, buf, (pl.ds(a, 2), pl.ds(2 * k, 2)), SEM_W + i)]
             for i, (hbm, buf) in enumerate(((wuv_hbm, wuv_buf), (wuk_hbm, wuk_buf), (wq_hbm, wq_buf)))
             for a in (0, 2)]
        units += w if k % 32 < LATE else [ffn_unit(k, -1, 1), w[0], ffn_unit(k, 3, 5)] + w[1:]
    c0 = len(units) // 2
    units += [c_unit(k, a) for k in range(B * 64) for a in range(0, C_RUNS, 2)]
    o0 = len(units) // 2
    for k in range(32):
        part = sum(k >= cut for cut in MXU_CUTS[1:]) + max(k - MXU_CUTS[-1], 0)
        lo, hi = 16 * k, 16 * k + 4 * D
        if k < LATE:
            units += [ffn_unit(k, 0, 2), o_unit(part, 0, 2, hi, 16), ffn_unit(k, 4, 6), o_unit(part, 2, 2, hi, 16),
                      ffn_unit(k, 1, 3), o_unit(part, 0, 2, lo, 16), ffn_unit(k, 5), o_unit(part, 2, 2, lo, 16)]
        else:
            units += [o_unit(part, 0, 2, hi, 16), o_unit(part, 0, 2, lo, 16),
                      o_unit(part, 2, 1, hi, 16), o_unit(part, 2, 2, lo, 16)]
    row = 4 * D + 16 * LATE
    for i, n in enumerate(END_UNITS):
        units.append(o_unit(part + 1 + i // 2, 3, 1, row, n))
        row += n
    queue0, queue1 = units[0::2], units[1::2]
    for i, group in enumerate(END_TINY):
        queue1 += [o_unit(O_PARTS - len(END_TINY) + i, 3, 1, row + 8 * r, 8, col, M // 2)
                   for r in group for col in (0, M // 2)]

    def start(unit, queue):
        for piece in unit:
            copy(*piece).start(priority=queue)

    def issue(lo, hi):
        for i in range(lo, hi):
            start(queue0[i], 0)
            if i + LEAD < len(queue1):
                start(queue1[i + LEAD], 1)

    def issue_c(lo, hi):
        def body(k):
            for i in range(4):
                start(c_unit(k, 4 * i), 0)
                start(c_unit(k + (i + LEAD) // 4, 4 * ((i + LEAD) % 4) + 2), 1)
        _loop(lo, hi, body)

    x_copy, b1_copy, b2_copy, o_copy = [
        pltpu.make_async_copy(src, dst, sems.at[SEM_SMALL + i])
        for i, (src, dst) in enumerate(((x_hbm, x_buf), (b1_hbm, b1_buf), (b2_hbm, b2_buf), (o_buf, o_hbm)))]

    for i in range(LEAD + 2):
        if i in (2, 16):
            start(queue0[i // 16], 0)
        start(queue1[i], 1)
    issue(2, 40)
    for i, c in enumerate((x_copy, b1_copy, b2_copy)):
        c.start()
        issue(40 + i, 41 + i)
    issue(43, 80)

    x_copy.wait()
    x = x_buf[...].astype(F32)
    xc = x - jnp.mean(x, axis=-1, keepdims=True)
    var = jnp.mean(xc * xc, axis=-1, keepdims=True)
    xn = (xc * lax.rsqrt(var + 1e-5)).astype(BF16)
    xf = xn.astype(F32)
    for b in range(B):
        for j in range(M // 128):
            cols = slice(j * 128, (j + 1) * 128)
            xs[b, cols, :] = jnp.broadcast_to(xf[b:b + 1, cols], (128, 128)).T
    e_buf[...] = (lax.broadcasted_iota(jnp.int32, (128, 1024), 1) // 8
                  == lax.broadcasted_iota(jnp.int32, (128, 1024), 0)).astype(F32).astype(BF16)
    issue(80, c0)
    issue_c(0, 10)

    wait_filled(wuv_buf, SEM_W)
    wait_filled(wuk_buf, SEM_W + 1)
    wait_filled(wq_buf, SEM_W + 2)

    def q_body(i, carry):
        q0, q1 = carry
        for u in range(8):
            m = pl.ds(i * 8 + u, 1)
            w = wq_buf[i >> 4, (i & 15) * 8 + u].astype(F32)
            q0 = q0 + xs[0, m, :] * w
            q1 = q1 + xs[1, m, :] * w
        return q0, q1

    def q_half(i, carry):
        carry = lax.fori_loop(i * 32, i * 32 + 32, q_body, carry)
        issue_c(10 + i * 4, 14 + i * 4)
        return carry

    q0, q1 = lax.fori_loop(0, 2, q_half, (jnp.zeros((H, D), F32), jnp.zeros((H, D), F32)))
    q = jnp.concatenate([q0, q1, jnp.zeros((128 - B * H, D), F32)], axis=0).astype(BF16)

    group = (lax.broadcasted_iota(jnp.int32, (16, 8, 128), 2) % H) // 8

    def qa_body(i):
        for u in range(8):
            w = wuk_buf[i, pl.ds(u * 16, 16)].reshape(16 * H, D)
            r = lax.dot_general(w, q, NT, preferred_element_type=F32).reshape(16, 4, 8, 128)
            v = jnp.where(group == 0, r[:, 0],
                          jnp.where(group == 1, r[:, 1], jnp.where(group == 2, r[:, 2], r[:, 3])))
            t8[pl.ds(pl.multiple_of((i * 8 + u) * 128, 128), 128), :] = v.reshape(128, 128)
        issue_c(18 + i * 3, 21 + i * 3)

    _loop(0, 4, qa_body)
    sub = lax.broadcasted_iota(jnp.int32, (128, 128), 1) % 8
    for j in range(DC // 128):
        t = t8[pl.ds(j * 1024, 128, stride=8), :]
        for s in range(1, 8):
            t = jnp.where(sub == s, t8[pl.ds(j * 1024 + s, 128, stride=8), :], t)
        qa_ref[:, j * 128:(j + 1) * 128] = (t.T[:B * H] * (D ** -0.5 * LOG2E)).astype(BF16)

    def issued(i):
        return jnp.maximum(jnp.where(i < BLOCKS, 36, 38) + 6 * i, 17 + 8 * i)

    def attention(b):
        heads = pl.ds(pl.multiple_of(b * H, H), H)
        m_ref[...] = jnp.full((H, 128), -jnp.inf, F32)
        l_ref[...] = jnp.zeros((H, 128), F32)
        acc_ref[...] = jnp.zeros((H, DC), F32)

        def block(g):
            i = b * BLOCKS + g
            pl.when(i < 14)(lambda: issue_c(jnp.where(i == BLOCKS, 84, issued(i - 1)), issued(i)))
            pl.when(i == 14)(lambda: issue(c0 + 4 * 121, o0 + 4))
            pl.when(i == 15)(lambda: issue(o0 + 16, o0 + 28))
            runs, rows = pl.ds(b * C_RUNS, C_RUNS), pl.ds(pl.multiple_of(g * 128, 128), 128)
            wait_filled(c_buf.at[runs, rows], SEM_C + i)
            sc = lax.dot_general(qa_ref[heads, :], c_buf[runs, rows].reshape(C_RUNS * 128, DC), NT,
                                 preferred_element_type=F32)
            m_prev = m_ref[...]
            m_new = jnp.maximum(m_prev, jnp.max(sc, axis=1, keepdims=True))
            p = jnp.exp2(sc - m_new[:, :1])
            alpha = jnp.exp2(m_prev - m_new)
            l_ref[...] = alpha * l_ref[...] + jnp.sum(p, axis=1, keepdims=True)
            m_ref[...] = m_new
            p = p.astype(BF16)
            pl.when(i == 14)(lambda: issue(o0 + 4, o0 + 16))
            pl.when(i == 15)(lambda: issue(o0 + 28, o0 + 42))
            pv = jnp.dot(p, c_buf[runs, rows].reshape(C_RUNS * 128, DC), preferred_element_type=F32)
            acc_ref[...] = acc_ref[...] * alpha[:, :1] + pv

        _loop(0, BLOCKS, block)
        pl.when(b == 0)(lambda: issue_c(78, 82))
        pl.when(b == 1)(lambda: issue(o0 + 42, o0 + 52))

        pc = (acc_ref[...] / l_ref[...][:, :1]).astype(BF16)
        pc = jnp.concatenate([pc[:, j * 128:(j + 1) * 128] for j in range(DC // 128)], axis=0)
        diag = (lax.broadcasted_iota(jnp.int32, (128, 1024), 1) % 8
                == lax.broadcasted_iota(jnp.int32, (128, 1024), 0) % 8)
        a = jnp.where(diag, jnp.dot(pc, e_buf[...], preferred_element_type=F32), 0.0)
        ctx = []
        for h in range(0, H, 8):
            if h == H // 2:
                pl.when(b == 0)(lambda: issue_c(82, 84))
                pl.when(b == 1)(lambda: issue(o0 + 52, o0 + 60))
            lhs = jnp.concatenate([a[j * H + h:j * H + h + 8] for j in range(DC // 128)], axis=1)
            ctx.append(jnp.dot(lhs.astype(BF16), wuv_buf[:, :, h:h + 8].reshape(DC * 8, D),
                               preferred_element_type=F32))
        ctx = jnp.concatenate(ctx, axis=0).astype(BF16).astype(F32)
        ctx_ref[heads] = ctx
        for k, h in enumerate(VPU_HEADS):
            mul_ref[b, k * D:(k + 1) * D] = jnp.broadcast_to(ctx[h:h + 1], (128, 128)).T

    _loop(0, B, attention)

    def wait_part(i):
        for piece in o_parts[i]:
            copy(*piece).wait()

    def spans(lo, hi):
        return [(h // 2, h % 2 * 4 * D + r, min(16 * hi, r // D * D + D) - r)
                for h in range(8 if lo < LATE else 7)
                for r in range(16 * lo, 16 * hi, 16) if r == 16 * lo or r % D == 0]

    groups = [spans(lo, hi) for lo, hi in zip(MXU_CUTS, MXU_CUTS[1:])]
    positions = (o0 + 60, o0 + 68, o0 + 84, len(queue0), len(queue0))
    issue(*positions[:2])
    lhs = [jnp.concatenate([ctx_ref[pl.ds(a * 8 + r // D, B, stride=H), :][:, r % D:r % D + n]
                            for a, r, n in group], axis=1).astype(BF16) for group in groups]
    s = jnp.zeros((B, M), F32)
    for i, group in enumerate(groups):
        if i > 0:
            issue(*positions[i:i + 2])
        wait_part(i)
        rhs = jnp.concatenate([wo_buf[a, r:r + n] for a, r, n in group], axis=0)
        s = s + jnp.dot(lhs[i], rhs, preferred_element_type=F32)
        if MXU_CUTS[i + 1] == LATE:
            wait_filled(w1_buf, SEM_FFN)
            wait_filled(w2_buf, SEM_FFN + 1)
            b1_copy.wait()
            b2_copy.wait()
            w1 = w1_buf[...].reshape(M // 8, F // 128, 8, 128)
            w1 = jnp.concatenate([w1[:, j].reshape(M, 128) for j in range(F // 128)], axis=1)
            hid = jnp.dot(xn, w1, preferred_element_type=F32) + b1_buf[...].astype(F32).reshape(1, F)
            hid = jax.nn.gelu(hid, approximate=True).astype(BF16)
            z = jnp.dot(hid, w2_buf[...], preferred_element_type=F32) + b2_buf[...].astype(F32).reshape(1, M)
            z8 = _rows8(z)
            g8 = z8 * jax.nn.sigmoid(z8)
    base8 = _rows8(x) + _rows8(s) * g8

    sublane = lax.broadcasted_iota(jnp.int32, (8, 128), 0)
    upper = {k: (sublane & k) != 0 for k in (1, 2, 4)}
    part, terms = None, None
    for i in range(len(groups), O_PARTS):
        wait_part(i)
        for _, _, (runs, rows, cols), _ in o_parts[i]:
            if cols.start:
                continue
            for a in range(runs.start, runs.start + runs.size):
                for r in range(rows.start, rows.start + rows.size, 8):
                    w = wo_buf[a, r:r + 8].astype(F32)
                    part = terms if part is None else [p + t for p, t in zip(part, terms)]
                    at = pl.ds(VPU_HEADS.index(a * 8 + r // D) * D + r % D, 8)
                    mul = [mul_ref[b, at, :] for b in range(B)]
                    terms = [w[:, j * 128:(j + 1) * 128] * mul[b] for j in range(M // 128) for b in range(B)]
    part = [p + t for p, t in zip(part, terms)]

    part = [jnp.where(upper[4], hi, lo) + pltpu.roll(jnp.where(upper[4], lo, hi), 4, 0)
            for lo, hi in zip(part[:4], part[4:])]
    for k in (2, 1):
        part = [jnp.where(upper[k], hi, lo) + jnp.where(upper[k], pltpu.roll(hi, k, 0), pltpu.roll(lo, 8 - k, 0))
                for lo, hi in zip(part[:k], part[k:])]
    o_buf[...] = (base8 + g8 * part[0]).astype(BF16)
    o_copy.start()
    o_copy.wait()


@jax.jit
def pallas_recurrent_scan__compressed_kv_cla__dense_activation_gelu__decode_kernel(
    A_x: jax.Array,
    A_c_kv: jax.Array,
    A_w_q: jax.Array,
    A_w_uk: jax.Array,
    A_w_uv: jax.Array,
    A_w_o: jax.Array,
    B_x: jax.Array,
    B_w1: jax.Array,
    B_b1: jax.Array,
    B_w2: jax.Array,
    B_b2: jax.Array,
):
    del B_x
    hbm = pl.BlockSpec(memory_space=pltpu.HBM)
    w1_tiles = B_w1.reshape(M // 8, 8, F // 128, 128).transpose(0, 2, 1, 3).reshape(W1_VIEW)
    out = pl.pallas_call(
        _kernel,
        out_shape=jax.ShapeDtypeStruct((8, 128), BF16),
        in_specs=[hbm] * 10,
        out_specs=hbm,
        scratch_shapes=[
            pltpu.VMEM(C_VIEW, BF16), pltpu.VMEM(W_VIEW, BF16), pltpu.VMEM(W_VIEW, BF16),
            pltpu.VMEM(W_VIEW, BF16), pltpu.VMEM(O_VIEW, BF16),
            pltpu.VMEM(W1_VIEW, BF16), pltpu.VMEM((F, M), BF16),
            pltpu.VMEM((B, M, 128), F32), pltpu.VMEM((DC * 8 + 8, 128), F32),
            pltpu.VMEM((B * H, DC), BF16), pltpu.VMEM((H, DC), F32),
            pltpu.VMEM((H, 128), F32), pltpu.VMEM((H, 128), F32),
            pltpu.VMEM((128, 1024), BF16),
            pltpu.VMEM((3 * H, D), F32), pltpu.VMEM((B, len(VPU_HEADS) * D, 128), F32),
            pltpu.VMEM((8, 128), BF16),
            pltpu.VMEM((F,), BF16), pltpu.VMEM((B, M), BF16), pltpu.VMEM((M,), BF16),
            pltpu.SemaphoreType.DMA((SEM_O + O_PARTS,)),
        ],
        compiler_params=pltpu.CompilerParams(
            vmem_limit_bytes=100 * 1024 * 1024, disable_semaphore_checks=True, disable_bounds_checks=True),
    )(A_x.reshape(B, M), A_c_kv.reshape(C_VIEW), A_w_q.reshape(W_VIEW), A_w_uk.reshape(W_VIEW),
      A_w_uv.reshape(W_VIEW), A_w_o.reshape(O_VIEW), w1_tiles, B_b1, B_w2, B_b2)
    return out.reshape(M // 128, B, 128).transpose(1, 0, 2).reshape(B, 1, M)
```

```python
import jax
import jax.numpy as jnp
from jax import lax
import jax.experimental.pallas as pl
import jax.experimental.pallas.tpu as pltpu

F32 = jnp.float32
BF16 = jnp.bfloat16

B, H, SK, D, M, DC, F = 2, 32, 16384, 128, 512, 512, 1792
LOG2E = 1.4426950408889634
NN = (((1,), (0,)), ((), ()))
NT = (((1,), (1,)), ((), ()))

LEAD = 26
W_VIEW = (4, 128, H, D)
C_RUNS = 16
C_VIEW = (B * C_RUNS, SK // C_RUNS, DC)
C_GROUPS = (2, 10, 18, 26, 32)
O_VIEW = (4, 8 * D, M)
W1_VIEW = (M // 8 * F // 128, 8, 128)
BLOCKS = 8
LATE = 20
MXU_CUTS = (0, 8, 16, LATE, 26)
END_UNITS = (24, 8) * 3
END_TINY = ((0, 4, 8, 1), (5, 9, 2), (6, 10), (3, 7), (11,))
VPU_HEADS = tuple(range(3, H - 4, 4)) + tuple(range(H - 4 + LATE // 8, H))
SEM_W, SEM_FFN, SEM_SMALL, SEM_C = 0, 3, 5, 9
SEM_O = SEM_C + B * BLOCKS
O_PARTS = len(MXU_CUTS) - 1 + 32 - MXU_CUTS[-1] + len(END_UNITS) // 2 + len(END_TINY)


def _loop(lo, hi, body):
    lax.fori_loop(lo, hi, lambda i, _: body(i), None)


def _rows8(v):
    return jnp.concatenate([v[:, j * 128:(j + 1) * 128] for j in range(M // 128)], axis=0)


def _kernel(x_hbm, ckv_hbm, wq_hbm, wuk_hbm, wuv_hbm, wo_hbm, w1_hbm, b1_hbm, w2_hbm, b2_hbm,
            o_hbm,
            c_buf, wq_buf, wuk_buf, wuv_buf, wo_buf, w1_buf, w2_buf,
            qa_ref, acc_ref, m_ref, l_ref, e_buf, ctx_ref, mul_ref, o_buf, b1_buf, x_buf, b2_buf,
            sems):
    def copy(hbm, buf, idx, sem):
        return pltpu.make_async_copy(hbm.at[idx], buf.at[idx], sems.at[sem])

    def wait_filled(buf, sem):
        pltpu.make_async_copy(buf, buf, sems.at[sem]).wait()

    def ffn_unit(k, *halves):
        n = F // 16
        return [(w2_hbm, w2_buf, pl.ds(16 * i, 16), SEM_FFN + 1) if i < n else
                (w1_hbm, w1_buf, pl.ds(8 * (i - n), 8), SEM_FFN)
                for i in [32 * h + k for h in halves] if i >= 0]

    def c_units(k, lo, hi):
        return [[(ckv_hbm, c_buf, (pl.ds(a, 2), pl.ds(16 * k, 16)), SEM_C + a // C_RUNS * BLOCKS + k // 8)]
                for a in range(lo, hi, 2)]

    o_parts = [[] for _ in range(O_PARTS)]

    def o_unit(part, a, runs, row, rows, col=0, cols=M):
        piece = (wo_hbm, wo_buf, (pl.ds(a, runs), pl.ds(row, rows), pl.ds(col, cols)), SEM_O + part)
        o_parts[part].append(piece)
        return [piece]

    units = []

    def sweep(lo, hi, groups):
        for k in range(lo, hi, 2):
            for first, second in zip(groups(k), groups(k + 1)):
                units.extend(first + second)

    def w_groups(k):
        w = [[(hbm, buf, (pl.ds(a, 2), pl.ds(2 * k, 2)), SEM_W + i)]
             for i, (hbm, buf) in enumerate(((wuv_hbm, wuv_buf), (wuk_hbm, wuk_buf), (wq_hbm, wq_buf)))
             for a in (0, 2)] + c_units(k, 0, C_GROUPS[0])
        if k % 32 < LATE:
            return w[:3], w[3:]
        return [ffn_unit(k, -1, 1), w[0], ffn_unit(k, 3, 5), w[1]], w[2:]

    def o_groups(k):
        part = sum(k >= cut for cut in MXU_CUTS[1:])
        lo, hi = 16 * k, 16 * k + 4 * D
        if k < LATE:
            return ([ffn_unit(k, 0, 2), o_unit(part, 0, 2, hi, 16), ffn_unit(k, 4, 6), o_unit(part, 2, 2, hi, 16)],
                    [ffn_unit(k, 1, 3), o_unit(part, 0, 2, lo, 16), ffn_unit(k, 5), o_unit(part, 2, 2, lo, 16)])
        part += max(k // 2 * 2 - MXU_CUTS[-1], 0)
        other = part + (k >= MXU_CUTS[-1])
        return ([o_unit(part, 2, 1, hi, 16), o_unit(part, 0, 2, hi, 16)],
                [o_unit(other, 0, 2, lo, 16), o_unit(other, 2, 2, lo, 16)])

    sweep(0, 64, w_groups)
    c0 = len(units) // 2
    c_ends = []
    for b in range(B):
        lo, mid, hi = C_GROUPS[2 * b:2 * b + 3]
        for g in range(BLOCKS):
            sweep(8 * g, 8 * g + 8, lambda k: (c_units(k, lo, mid), c_units(k, mid, hi)))
            c_ends.append(len(units) // 2)
    o0 = len(units) // 2
    sweep(0, 32, o_groups)
    row = 4 * D + 16 * LATE
    for i, n in enumerate(END_UNITS):
        units.append(o_unit(O_PARTS - len(END_TINY) - len(END_UNITS) // 2 + i // 2, 3, 1, row, n))
        row += n
    queue0, queue1 = units[0::2], units[1::2]
    for i, group in enumerate(END_TINY):
        queue1 += [o_unit(O_PARTS - len(END_TINY) + i, 3, 1, row + 8 * r, 8, col, M // 2)
                   for r in group for col in (0, M // 2)]

    def start(unit, queue):
        for piece in unit:
            copy(*piece).start(priority=queue)

    def issue(lo, hi):
        for i in range(lo, hi):
            start(queue0[i], 0)
            if i + LEAD < len(queue1):
                start(queue1[i + LEAD], 1)

    def issue_nth(i, ranges, first=0):
        n = len(ranges) // 2
        if n == 0:
            issue(*ranges[0])
        else:
            pl.when(i < first + n)(lambda: issue_nth(i, ranges[:n], first))
            pl.when(i >= first + n)(lambda: issue_nth(i, ranges[n:], first + n))

    issued = [2]

    def take(count, upto=0):
        issued.append(min(max(issued[-1] + count, upto), len(queue0)))
        return issued[-2:]

    x_copy, b1_copy, b2_copy, o_copy = [
        pltpu.make_async_copy(src, dst, sems.at[SEM_SMALL + i])
        for i, (src, dst) in enumerate(((x_hbm, x_buf), (b1_hbm, b1_buf), (b2_hbm, b2_buf), (o_buf, o_hbm)))]

    for i in range(LEAD + 2):
        if i in (2, 16):
            start(queue0[i // 16], 0)
        start(queue1[i], 1)
    for c in (x_copy, b1_copy, b2_copy):
        issue(*take(20))
        c.start()
    issue(*take(20))

    x_copy.wait()
    x = x_buf[...].astype(F32)
    xc = x - jnp.mean(x, axis=-1, keepdims=True)
    var = jnp.mean(xc * xc, axis=-1, keepdims=True)
    xn = xc * lax.rsqrt(var + 1e-5)

    def heads8(w_buf, h):
        return w_buf[:, :, pl.ds(h, 8)].reshape(512 * 8, D)

    def own_head(v):
        return jnp.where(lax.broadcasted_iota(jnp.int32, v.shape, 1) % 8
                         == lax.broadcasted_iota(jnp.int32, v.shape, 0) % 8, v, 0.0)

    def by_quarters(v, dims):
        n, m = v.shape[0], v.shape[1] // 4
        v = jnp.concatenate([v[:, j * m:(j + 1) * m] for j in range(4)], axis=0).astype(BF16)
        v = lax.dot_general(v, e_buf[...], dims, preferred_element_type=F32)
        return jnp.concatenate([v[j * n:(j + 1) * n] for j in range(4)], axis=1)

    e_buf[...] = (lax.broadcasted_iota(jnp.int32, (128, 1024), 1) // 8
                  == lax.broadcasted_iota(jnp.int32, (128, 1024), 0)).astype(F32).astype(BF16)
    xs = jnp.concatenate([jnp.broadcast_to(xn[b:b + 1], (8, M)) for b in range(B)], axis=0)
    xs = own_head(by_quarters(xs, NN)).astype(BF16)
    issue(*take(0, c0 + 40))

    wait_filled(wuv_buf, SEM_W)
    wait_filled(wuk_buf, SEM_W + 1)
    wait_filled(wq_buf, SEM_W + 2)
    after_qa = [take(12) for _ in range(H // 8)]

    def absorb(i):
        h = pl.multiple_of(i * 8, 8)
        q = jnp.dot(xs, heads8(wq_buf, h), preferred_element_type=F32).astype(BF16)
        r = lax.dot_general(q, heads8(wuk_buf, h), NT, preferred_element_type=F32)
        qa = by_quarters(own_head(r * (D ** -0.5 * LOG2E)), NT)
        for b in range(B):
            qa_ref[b, pl.ds(h, 8)] = qa[b * 8:(b + 1) * 8]
        issue_nth(i, after_qa)

    _loop(0, H // 8, absorb)

    before, during, ctx_before, ctx_during = [], [], [], []
    for i, end in enumerate(c_ends):
        before.append(take(9, end + (36 if end < o0 else 28)))
        during.append(take(16))
        if i % BLOCKS == BLOCKS - 1:
            ctx_before.append(take(8))
            ctx_during.append(take(10))

    def attention(b):
        m_ref[...] = jnp.full((H, 128), -jnp.inf, F32)
        l_ref[...] = jnp.zeros((H, 128), F32)
        acc_ref[...] = jnp.zeros((H, DC), F32)

        def block(g):
            i = b * BLOCKS + g
            issue_nth(i, before)
            runs, rows = pl.ds(b * C_RUNS, C_RUNS), pl.ds(pl.multiple_of(g * 128, 128), 128)
            wait_filled(c_buf.at[runs, rows], SEM_C + i)
            sc = lax.dot_general(qa_ref[b].astype(BF16), c_buf[runs, rows].reshape(C_RUNS * 128, DC), NT,
                                 preferred_element_type=F32)
            m_prev = m_ref[...]
            m_new = jnp.maximum(m_prev, jnp.max(sc, axis=1, keepdims=True))
            p = jnp.exp2(sc - m_new[:, :1])
            alpha = jnp.exp2(m_prev - m_new)
            l_ref[...] = alpha * l_ref[...] + jnp.sum(p, axis=1, keepdims=True)
            m_ref[...] = m_new
            p = p.astype(BF16)
            issue_nth(i, during)
            pv = jnp.dot(p, c_buf[runs, rows].reshape(C_RUNS * 128, DC), preferred_element_type=F32)
            acc_ref[...] = acc_ref[...] * alpha[:, :1] + pv

        _loop(0, BLOCKS, block)
        issue_nth(b, ctx_before)

        pc = own_head(by_quarters(acc_ref[...] / l_ref[...][:, :1], NN))
        ctx = []
        for h in range(0, H, 8):
            if h == H // 2:
                issue_nth(b, ctx_during)
            ctx.append(jnp.dot(pc[h:h + 8].astype(BF16), heads8(wuv_buf, h), preferred_element_type=F32))
        ctx = jnp.concatenate(ctx, axis=0).astype(BF16).astype(F32)
        ctx_ref[pl.ds(pl.multiple_of(b * H, H), H)] = ctx
        for k, h in enumerate(VPU_HEADS):
            mul_ref[b, k * D:(k + 1) * D] = jnp.broadcast_to(ctx[h:h + 1], (128, 128)).T

    _loop(0, B, attention)

    def wait_part(i):
        for piece in o_parts[i]:
            copy(*piece).wait()

    def spans(lo, hi):
        return [(h // 2, h % 2 * 4 * D + r, min(16 * hi, r // D * D + D) - r)
                for h in range(8 if lo < LATE else 7)
                for r in range(16 * lo, 16 * hi, 16) if r == 16 * lo or r % D == 0]

    groups = [spans(lo, hi) for lo, hi in zip(MXU_CUTS, MXU_CUTS[1:])]
    issue(*take(8))
    lhs = [jnp.concatenate([ctx_ref[pl.ds(a * 8 + r // D, B, stride=H), :][:, r % D:r % D + n]
                            for a, r, n in group], axis=1).astype(BF16) for group in groups]
    s = jnp.zeros((B, M), F32)
    for i, group in enumerate(groups):
        issue(*take(0, o0 + 4 * MXU_CUTS[i + 1] + 28))
        wait_part(i)
        rhs = jnp.concatenate([wo_buf[a, r:r + n] for a, r, n in group], axis=0)
        s = s + jnp.dot(lhs[i], rhs, preferred_element_type=F32)
        if MXU_CUTS[i + 1] == LATE:
            wait_filled(w1_buf, SEM_FFN)
            wait_filled(w2_buf, SEM_FFN + 1)
            b1_copy.wait()
            b2_copy.wait()
            w1 = w1_buf[...].reshape(M // 8, F // 128, 8, 128)
            w1 = jnp.concatenate([w1[:, j].reshape(M, 128) for j in range(F // 128)], axis=1)
            hid = jnp.dot(xn.astype(BF16), w1, preferred_element_type=F32) + b1_buf[...].astype(F32).reshape(1, F)
            hid = jax.nn.gelu(hid, approximate=True).astype(BF16)
            z = jnp.dot(hid, w2_buf[...], preferred_element_type=F32) + b2_buf[...].astype(F32).reshape(1, M)
            z8 = _rows8(z)
            g8 = z8 * jax.nn.sigmoid(z8)
    assert issued[-1] == len(queue0) >= len(queue1) - LEAD
    base8 = _rows8(x) + _rows8(s) * g8

    sublane = lax.broadcasted_iota(jnp.int32, (8, 128), 0)
    upper = {k: (sublane & k) != 0 for k in (1, 2, 4)}
    part, terms = None, None
    for i in range(len(groups), O_PARTS):
        wait_part(i)
        for _, _, (runs, rows, cols), _ in o_parts[i]:
            if cols.start:
                continue
            for a in range(runs.start, runs.start + runs.size):
                for r in range(rows.start, rows.start + rows.size, 8):
                    w = wo_buf[a, r:r + 8].astype(F32)
                    part = terms if part is None else [p + t for p, t in zip(part, terms)]
                    at = pl.ds(VPU_HEADS.index(a * 8 + r // D) * D + r % D, 8)
                    mul = [mul_ref[b, at, :] for b in range(B)]
                    terms = [w[:, j * 128:(j + 1) * 128] * mul[b] for j in range(M // 128) for b in range(B)]
    part = [p + t for p, t in zip(part, terms)]

    part = [jnp.where(upper[4], hi, lo) + pltpu.roll(jnp.where(upper[4], lo, hi), 4, 0)
            for lo, hi in zip(part[:4], part[4:])]
    for k in (2, 1):
        part = [jnp.where(upper[k], hi, lo) + jnp.where(upper[k], pltpu.roll(hi, k, 0), pltpu.roll(lo, 8 - k, 0))
                for lo, hi in zip(part[:k], part[k:])]
    o_buf[...] = (base8 + g8 * part[0]).astype(BF16)
    o_copy.start()
    o_copy.wait()


@jax.jit
def pallas_recurrent_scan__compressed_kv_cla__dense_activation_gelu__decode_kernel(
    A_x: jax.Array,
    A_c_kv: jax.Array,
    A_w_q: jax.Array,
    A_w_uk: jax.Array,
    A_w_uv: jax.Array,
    A_w_o: jax.Array,
    B_x: jax.Array,
    B_w1: jax.Array,
    B_b1: jax.Array,
    B_w2: jax.Array,
    B_b2: jax.Array,
):
    del B_x
    hbm = pl.BlockSpec(memory_space=pltpu.HBM)
    w1_tiles = B_w1.reshape(M // 8, 8, F // 128, 128).transpose(0, 2, 1, 3).reshape(W1_VIEW)
    out = pl.pallas_call(
        _kernel,
        out_shape=jax.ShapeDtypeStruct((8, 128), BF16),
        in_specs=[hbm] * 10,
        out_specs=hbm,
        scratch_shapes=[
            pltpu.VMEM(C_VIEW, BF16), pltpu.VMEM(W_VIEW, BF16), pltpu.VMEM(W_VIEW, BF16),
            pltpu.VMEM(W_VIEW, BF16), pltpu.VMEM(O_VIEW, BF16),
            pltpu.VMEM(W1_VIEW, BF16), pltpu.VMEM((F, M), BF16),
            pltpu.VMEM((B, H, DC), F32), pltpu.VMEM((H, DC), F32),
            pltpu.VMEM((H, 128), F32), pltpu.VMEM((H, 128), F32),
            pltpu.VMEM((128, 1024), BF16),
            pltpu.VMEM((3 * H, D), F32), pltpu.VMEM((B, len(VPU_HEADS) * D, 128), F32),
            pltpu.VMEM((8, 128), BF16),
            pltpu.VMEM((F,), BF16), pltpu.VMEM((B, M), BF16), pltpu.VMEM((M,), BF16),
            pltpu.SemaphoreType.DMA((SEM_O + O_PARTS,)),
        ],
        compiler_params=pltpu.CompilerParams(
            vmem_limit_bytes=100 * 1024 * 1024, disable_semaphore_checks=True, disable_bounds_checks=True),
    )(A_x.reshape(B, M), A_c_kv.reshape(C_VIEW), A_w_q.reshape(W_VIEW), A_w_uk.reshape(W_VIEW),
      A_w_uv.reshape(W_VIEW), A_w_o.reshape(O_VIEW), w1_tiles, B_b1, B_w2, B_b2)
    return out.reshape(M // 128, B, 128).transpose(1, 0, 2).reshape(B, 1, M)
```

```python
import jax
import jax.numpy as jnp
from jax import lax
import jax.experimental.pallas as pl
import jax.experimental.pallas.tpu as pltpu

F32 = jnp.float32
BF16 = jnp.bfloat16

B, H, SK, D, M, DC, F = 2, 32, 16384, 128, 512, 512, 1792
LOG2E = 1.4426950408889634
NN = (((1,), (0,)), ((), ()))
NT = (((1,), (1,)), ((), ()))

LEAD = 26
W_VIEW = (4, 128, H, D)
C_RUNS = 16
C_VIEW = (B * C_RUNS, SK // C_RUNS, DC)
C_GROUPS = (2, 10, 18, 26, 32)
O_VIEW = (4, 8 * D, M)
W1_VIEW = (M // 8 * F // 128, 8, 128)
BLOCKS = 8
LATE = 20
MXU_CUTS = (0, 8, 16, LATE, 26)
END_UNITS = (24, 8) * 3
END_TINY = ((0, 4, 8, 1), (5, 9, 2), (6, 10), (3, 7), (11,))
VPU_HEADS = tuple(range(3, H - 4, 4)) + tuple(range(H - 4 + LATE // 8, H))
SEM_W, SEM_FFN, SEM_SMALL, SEM_C = 0, 3, 5, 9
SEM_O = SEM_C + B * BLOCKS
ROUND_PARTS = len(MXU_CUTS) - 1 + 32 - MXU_CUTS[-1]
O_PARTS = ROUND_PARTS + len(END_UNITS) // 2 + len(END_TINY)


def _loop(lo, hi, body):
    lax.fori_loop(lo, hi, lambda i, _: body(i), None)


def _rows8(v):
    return jnp.concatenate([v[:, j * 128:(j + 1) * 128] for j in range(M // 128)], axis=0)


def _kernel(x_hbm, ckv_hbm, wq_hbm, wuk_hbm, wuv_hbm, wo_hbm, w1_hbm, b1_hbm, w2_hbm, b2_hbm,
            o_hbm,
            c_buf, wq_buf, wuk_buf, wuv_buf, wo_buf, w1_buf, w2_buf,
            qa_ref, acc_ref, m_ref, l_ref, e_buf, ctx_ref, mul_ref, o_buf, b1_buf, x_buf, b2_buf,
            sems):
    def copy(hbm, buf, idx, sem):
        return pltpu.make_async_copy(hbm.at[idx], buf.at[idx], sems.at[sem])

    def wait_filled(buf, sem):
        pltpu.make_async_copy(buf, buf, sems.at[sem]).wait()

    def ffn_unit(k, *halves):
        n = F // 16
        return [(w2_hbm, w2_buf, pl.ds(16 * i, 16), SEM_FFN + 1) if i < n else
                (w1_hbm, w1_buf, pl.ds(8 * (i - n), 8), SEM_FFN)
                for i in [32 * h + k for h in halves] if i >= 0]

    def c_units(k, lo, hi):
        return [[(ckv_hbm, c_buf, (pl.ds(a, 2), pl.ds(16 * k, 16)), SEM_C + a // C_RUNS * BLOCKS + k // 8)]
                for a in range(lo, hi, 2)]

    o_parts = [[] for _ in range(O_PARTS)]

    def o_unit(part, a, runs, row, rows, col=0, cols=M):
        piece = (wo_hbm, wo_buf, (pl.ds(a, runs), pl.ds(row, rows), pl.ds(col, cols)), SEM_O + part)
        o_parts[part].append(piece)
        return [piece]

    units = []

    def sweep(lo, hi, groups):
        for k in range(lo, hi, 2):
            for first, second in zip(groups(k), groups(k + 1)):
                units.extend(first + second)

    def w_groups(k):
        w = [[(hbm, buf, (pl.ds(a, 2), pl.ds(2 * k, 2)), SEM_W + i)]
             for i, (hbm, buf) in enumerate(((wuv_hbm, wuv_buf), (wuk_hbm, wuk_buf), (wq_hbm, wq_buf)))
             for a in (0, 2)] + c_units(k, 0, C_GROUPS[0])
        if k % 32 < LATE:
            return w[:3], w[3:]
        return [ffn_unit(k, -1, 1), w[0], ffn_unit(k, 3, 5), w[1]], w[2:]

    def o_groups(k):
        part = sum(k >= cut for cut in MXU_CUTS[1:])
        lo, hi = 16 * k, 16 * k + 4 * D
        if k < LATE:
            return ([ffn_unit(k, 0, 2), o_unit(part, 0, 2, hi, 16), ffn_unit(k, 4, 6), o_unit(part, 2, 2, hi, 16)],
                    [ffn_unit(k, 1, 3), o_unit(part, 0, 2, lo, 16), ffn_unit(k, 5), o_unit(part, 2, 2, lo, 16)])
        part += max(k // 2 * 2 - MXU_CUTS[-1], 0)
        other = part + (k >= MXU_CUTS[-1])
        return ([o_unit(part, 2, 1, hi, 16), o_unit(part, 0, 2, hi, 16)],
                [o_unit(other, 0, 2, lo, 16)], [o_unit(other, 2, 2, lo, 16)])

    sweep(0, 64, w_groups)
    c0 = len(units) // 2
    c_ends = []
    for b in range(B):
        lo, mid, hi = C_GROUPS[2 * b:2 * b + 3]
        for g in range(BLOCKS):
            sweep(8 * g, 8 * g + 8, lambda k: (c_units(k, lo, mid), c_units(k, mid, hi)))
            c_ends.append(len(units) // 2)
    o0 = len(units) // 2
    sweep(0, 32, o_groups)
    row = 4 * D + 16 * LATE
    for i, n in enumerate(END_UNITS):
        units.append(o_unit(ROUND_PARTS + i // 2, 3, 1, row, n))
        row += n
    queue0, queue1 = units[0::2], units[1::2]
    for i, group in enumerate(END_TINY):
        queue1 += [o_unit(O_PARTS - len(END_TINY) + i, 3, 1, row + 8 * r, 8, col, M // 2)
                   for r in group for col in (0, M // 2)]

    def start(unit, queue):
        for piece in unit:
            copy(*piece).start(priority=queue)

    def issue(lo, hi):
        for i in range(lo, hi):
            start(queue0[i], 0)
            if i + LEAD < len(queue1):
                start(queue1[i + LEAD], 1)

    def issue_nth(i, ranges, first=0):
        n = len(ranges) // 2
        if n == 0:
            issue(*ranges[0])
        else:
            pl.when(i < first + n)(lambda: issue_nth(i, ranges[:n], first))
            pl.when(i >= first + n)(lambda: issue_nth(i, ranges[n:], first + n))

    issued = [2]

    def take(count, upto=0):
        issued.append(min(max(issued[-1] + count, upto), len(queue0)))
        return issued[-2:]

    x_copy, b1_copy, b2_copy, o_copy = [
        pltpu.make_async_copy(src, dst, sems.at[SEM_SMALL + i])
        for i, (src, dst) in enumerate(((x_hbm, x_buf), (b1_hbm, b1_buf), (b2_hbm, b2_buf), (o_buf, o_hbm)))]

    for i in range(LEAD + 2):
        if i in (2, 16):
            start(queue0[i // 16], 0)
        start(queue1[i], 1)
    for c in (x_copy, b1_copy, b2_copy):
        issue(*take(20))
        c.start()
    issue(*take(20))

    x_copy.wait()
    x = x_buf[...].astype(F32)
    xc = x - jnp.mean(x, axis=-1, keepdims=True)
    var = jnp.mean(xc * xc, axis=-1, keepdims=True)
    xn = xc * lax.rsqrt(var + 1e-5)

    def heads8(w_buf, h):
        return w_buf[:, :, pl.ds(h, 8)].reshape(512 * 8, D)

    def own_head(v):
        return jnp.where(lax.broadcasted_iota(jnp.int32, v.shape, 1) % 8
                         == lax.broadcasted_iota(jnp.int32, v.shape, 0) % 8, v, 0.0)

    def by_quarters(v, dims):
        n, m = v.shape[0], v.shape[1] // 4
        v = jnp.concatenate([v[:, j * m:(j + 1) * m] for j in range(4)], axis=0).astype(BF16)
        v = lax.dot_general(v, e_buf[...], dims, preferred_element_type=F32)
        return jnp.concatenate([v[j * n:(j + 1) * n] for j in range(4)], axis=1)

    e_buf[...] = (lax.broadcasted_iota(jnp.int32, (128, 1024), 1) // 8
                  == lax.broadcasted_iota(jnp.int32, (128, 1024), 0)).astype(F32).astype(BF16)
    xs = jnp.concatenate([jnp.broadcast_to(xn[b:b + 1], (8, M)) for b in range(B)], axis=0)
    xs = own_head(by_quarters(xs, NN)).astype(BF16)
    issue(*take(0, c0 + 40))

    wait_filled(wuv_buf, SEM_W)
    wait_filled(wuk_buf, SEM_W + 1)
    wait_filled(wq_buf, SEM_W + 2)
    after_qa = [take(12) for _ in range(H // 8)]

    def absorb(i):
        h = pl.multiple_of(i * 8, 8)
        q = jnp.dot(xs, heads8(wq_buf, h), preferred_element_type=F32).astype(BF16)
        r = lax.dot_general(q, heads8(wuk_buf, h), NT, preferred_element_type=F32)
        qa = by_quarters(own_head(r * (D ** -0.5 * LOG2E)), NT)
        for b in range(B):
            qa_ref[b, pl.ds(h, 8)] = qa[b * 8:(b + 1) * 8]
        issue_nth(i, after_qa)

    _loop(0, H // 8, absorb)

    before, during, ctx_before, ctx_during = [], [], [], []
    for i, end in enumerate(c_ends):
        before.append(take(9, end + (36 if end < o0 else 28)))
        during.append(take(16))
        if i % BLOCKS == BLOCKS - 1:
            ctx_before.append(take(8))
            ctx_during.append(take(10))

    def attention(b):
        m_ref[...] = jnp.full((H, 128), -jnp.inf, F32)
        l_ref[...] = jnp.zeros((H, 128), F32)
        acc_ref[...] = jnp.zeros((H, DC), F32)

        def block(g):
            i = b * BLOCKS + g
            issue_nth(i, before)
            runs, rows = pl.ds(b * C_RUNS, C_RUNS), pl.ds(pl.multiple_of(g * 128, 128), 128)
            wait_filled(c_buf.at[runs, rows], SEM_C + i)
            sc = lax.dot_general(qa_ref[b].astype(BF16), c_buf[runs, rows].reshape(C_RUNS * 128, DC), NT,
                                 preferred_element_type=F32)
            m_prev = m_ref[...]
            m_new = jnp.maximum(m_prev, jnp.max(sc, axis=1, keepdims=True))
            p = jnp.exp2(sc - m_new[:, :1])
            alpha = jnp.exp2(m_prev - m_new)
            l_ref[...] = alpha * l_ref[...] + jnp.sum(p, axis=1, keepdims=True)
            m_ref[...] = m_new
            p = p.astype(BF16)
            issue_nth(i, during)
            pv = jnp.dot(p, c_buf[runs, rows].reshape(C_RUNS * 128, DC), preferred_element_type=F32)
            acc_ref[...] = acc_ref[...] * alpha[:, :1] + pv

        _loop(0, BLOCKS, block)
        issue_nth(b, ctx_before)

        pc = own_head(by_quarters(acc_ref[...] / l_ref[...][:, :1], NN))
        ctx = []
        for h in range(0, H, 8):
            if h == H // 2:
                issue_nth(b, ctx_during)
            ctx.append(jnp.dot(pc[h:h + 8].astype(BF16), heads8(wuv_buf, h), preferred_element_type=F32))
        ctx = jnp.concatenate(ctx, axis=0).astype(BF16).astype(F32)
        ctx_ref[pl.ds(pl.multiple_of(b * H, H), H)] = ctx
        for k, h in enumerate(VPU_HEADS):
            mul_ref[b, k * D:(k + 1) * D] = jnp.broadcast_to(ctx[h:h + 1], (128, 128)).T

    _loop(0, B, attention)

    def wait_part(i):
        for piece in o_parts[i]:
            copy(*piece).wait()

    def spans(lo, hi):
        return [(h // 2, h % 2 * 4 * D + r, min(16 * hi, r // D * D + D) - r)
                for h in range(8 if lo < LATE else 7)
                for r in range(16 * lo, 16 * hi, 16) if r == 16 * lo or r % D == 0]

    groups = [spans(lo, hi) for lo, hi in zip(MXU_CUTS, MXU_CUTS[1:])]
    issue(*take(8))
    lhs = [jnp.concatenate([ctx_ref[pl.ds(a * 8 + r // D, B, stride=H), :][:, r % D:r % D + n]
                            for a, r, n in group], axis=1).astype(BF16) for group in groups]
    s = jnp.zeros((B, M), F32)
    for i, group in enumerate(groups):
        issue(*take(0, o0 + 4 * MXU_CUTS[i + 1] + 28))
        wait_part(i)
        rhs = jnp.concatenate([wo_buf[a, r:r + n] for a, r, n in group], axis=0)
        s = s + jnp.dot(lhs[i], rhs, preferred_element_type=F32)
        if MXU_CUTS[i + 1] == LATE:
            wait_filled(w1_buf, SEM_FFN)
            wait_filled(w2_buf, SEM_FFN + 1)
            b1_copy.wait()
            b2_copy.wait()
            w1 = w1_buf[...].reshape(M // 8, F // 128, 8, 128)
            w1 = jnp.concatenate([w1[:, j].reshape(M, 128) for j in range(F // 128)], axis=1)
            hid = jnp.dot(xn.astype(BF16), w1, preferred_element_type=F32) + b1_buf[...].astype(F32).reshape(1, F)
            hid = jax.nn.gelu(hid, approximate=True).astype(BF16)
            z = jnp.dot(hid, w2_buf[...], preferred_element_type=F32) + b2_buf[...].astype(F32).reshape(1, M)
            z8 = _rows8(z)
            g8 = z8 * jax.nn.sigmoid(z8)
    assert issued[-1] == len(queue0) >= len(queue1) - LEAD
    base8 = _rows8(x) + _rows8(s) * g8

    sublane = lax.broadcasted_iota(jnp.int32, (8, 128), 0)
    upper = {k: (sublane & k) != 0 for k in (1, 2, 4)}
    part, terms = None, None
    for i in range(len(groups), O_PARTS):
        wait_part(i)
        for _, _, (runs, rows, cols), _ in o_parts[i]:
            if cols.start:
                continue
            for a in range(runs.start, runs.start + runs.size):
                for r in range(rows.start, rows.start + rows.size, 8):
                    w = wo_buf[a, r:r + 8].astype(F32)
                    part = terms if part is None else [p + t for p, t in zip(part, terms)]
                    at = pl.ds(VPU_HEADS.index(a * 8 + r // D) * D + r % D, 8)
                    mul = [mul_ref[b, at, :] for b in range(B)]
                    terms = [w[:, j * 128:(j + 1) * 128] * mul[b] for j in range(M // 128) for b in range(B)]
    part = [p + t for p, t in zip(part, terms)]

    part = [jnp.where(upper[4], hi, lo) + pltpu.roll(jnp.where(upper[4], lo, hi), 4, 0)
            for lo, hi in zip(part[:4], part[4:])]
    for k in (2, 1):
        part = [jnp.where(upper[k], hi, lo) + jnp.where(upper[k], pltpu.roll(hi, k, 0), pltpu.roll(lo, 8 - k, 0))
                for lo, hi in zip(part[:k], part[k:])]
    o_buf[...] = (base8 + g8 * part[0]).astype(BF16)
    o_copy.start()
    o_copy.wait()


@jax.jit
def pallas_recurrent_scan__compressed_kv_cla__dense_activation_gelu__decode_kernel(
    A_x: jax.Array,
    A_c_kv: jax.Array,
    A_w_q: jax.Array,
    A_w_uk: jax.Array,
    A_w_uv: jax.Array,
    A_w_o: jax.Array,
    B_x: jax.Array,
    B_w1: jax.Array,
    B_b1: jax.Array,
    B_w2: jax.Array,
    B_b2: jax.Array,
):
    del B_x
    hbm = pl.BlockSpec(memory_space=pltpu.HBM)
    w1_tiles = B_w1.reshape(M // 8, 8, F // 128, 128).transpose(0, 2, 1, 3).reshape(W1_VIEW)
    out = pl.pallas_call(
        _kernel,
        out_shape=jax.ShapeDtypeStruct((8, 128), BF16),
        in_specs=[hbm] * 10,
        out_specs=hbm,
        scratch_shapes=[
            pltpu.VMEM(C_VIEW, BF16), pltpu.VMEM(W_VIEW, BF16), pltpu.VMEM(W_VIEW, BF16),
            pltpu.VMEM(W_VIEW, BF16), pltpu.VMEM(O_VIEW, BF16),
            pltpu.VMEM(W1_VIEW, BF16), pltpu.VMEM((F, M), BF16),
            pltpu.VMEM((B, H, DC), F32), pltpu.VMEM((H, DC), F32),
            pltpu.VMEM((H, 128), F32), pltpu.VMEM((H, 128), F32),
            pltpu.VMEM((128, 1024), BF16),
            pltpu.VMEM((3 * H, D), F32), pltpu.VMEM((B, len(VPU_HEADS) * D, 128), F32),
            pltpu.VMEM((8, 128), BF16),
            pltpu.VMEM((F,), BF16), pltpu.VMEM((B, M), BF16), pltpu.VMEM((M,), BF16),
            pltpu.SemaphoreType.DMA((SEM_O + O_PARTS,)),
        ],
        compiler_params=pltpu.CompilerParams(
            vmem_limit_bytes=100 * 1024 * 1024, disable_semaphore_checks=True, disable_bounds_checks=True),
    )(A_x.reshape(B, M), A_c_kv.reshape(C_VIEW), A_w_q.reshape(W_VIEW), A_w_uk.reshape(W_VIEW),
      A_w_uv.reshape(W_VIEW), A_w_o.reshape(O_VIEW), w1_tiles, B_b1, B_w2, B_b2)
    return out.reshape(M // 128, B, 128).transpose(1, 0, 2).reshape(B, 1, M)
```

```python
import jax
import jax.numpy as jnp
from jax import lax
import jax.experimental.pallas as pl
import jax.experimental.pallas.tpu as pltpu

F32 = jnp.float32
BF16 = jnp.bfloat16

B, H, SK, D, M, DC, F = 2, 32, 16384, 128, 512, 512, 1792
LOG2E = 1.4426950408889634
NN = (((1,), (0,)), ((), ()))
NT = (((1,), (1,)), ((), ()))

LEAD = 26
W_VIEW = (4, 128, H, D)
C_RUNS = 16
C_VIEW = (B * C_RUNS, SK // C_RUNS, DC)
SHIFT = 46
GROUPS = ((-1, 7, 15, 23, 31, 35, 43), (0, 6, 14, 22, 30, 38, 44))
O_VIEW = (4, 8 * D, M)
W1_VIEW = (M // 8 * F // 128, 8, 128)
BLOCKS = 8
LATE = 20
MXU_CUTS = (0, 8, 16, LATE, 26)
END_UNITS = (24, 8) * 3
END_TINY = ((0, 4, 8, 1), (5, 9, 2), (6, 10), (3, 7), (11,))
VPU_HEADS = tuple(range(3, H - 4, 4)) + tuple(range(H - 4 + LATE // 8, H))
SEM_W, SEM_FFN, SEM_SMALL, SEM_C = 0, 3, 5, 9
SEM_O = SEM_C + B * BLOCKS
ROUND_PARTS = len(MXU_CUTS) - 1 + 32 - MXU_CUTS[-1]
O_PARTS = ROUND_PARTS + len(END_UNITS) // 2 + len(END_TINY)


def _loop(lo, hi, body):
    lax.fori_loop(lo, hi, lambda i, _: body(i), None)


def _rows8(v):
    return jnp.concatenate([v[:, j * 128:(j + 1) * 128] for j in range(M // 128)], axis=0)


def _kernel(x_hbm, ckv_hbm, wq_hbm, wuk_hbm, wuv_hbm, wo_hbm, w1_hbm, b1_hbm, w2_hbm, b2_hbm,
            o_hbm,
            c_buf, wq_buf, wuk_buf, wuv_buf, wo_buf, w1_buf, w2_buf,
            qa_ref, acc_ref, m_ref, l_ref, e_buf, ctx_ref, mul_ref, o_buf, b1_buf, x_buf, b2_buf,
            sems):
    def copy(hbm, buf, idx, sem):
        return pltpu.make_async_copy(hbm.at[idx], buf.at[idx], sems.at[sem])

    def wait_filled(buf, sem):
        pltpu.make_async_copy(buf, buf, sems.at[sem]).wait()

    def ffn_unit(k, *halves):
        n = F // 16
        return [(w2_hbm, w2_buf, pl.ds(16 * ((i + 1) % n), 16), SEM_FFN + 1) if i < n else
                (w1_hbm, w1_buf, pl.ds(8 * (i - n), 8), SEM_FFN)
                for i in [32 * h + k for h in halves] if i >= 0]

    def run_piece(k, a, runs):
        if a < 12:
            hbm, buf = ((wuv_hbm, wuv_buf), (wuk_hbm, wuk_buf), (wq_hbm, wq_buf))[a // 4]
            return hbm, buf, (pl.ds(a % 4, runs), pl.ds(2 * k, 2)), SEM_W + a // 4
        a -= 12
        return ckv_hbm, c_buf, (pl.ds(a, runs), pl.ds(16 * k, 16)), SEM_C + a // C_RUNS * BLOCKS + k // 8

    def run_groups(k, phase):
        ends = GROUPS[k >= SHIFT][2 * phase:2 * phase + 3]
        return [[[run_piece(k, a % 44, 1), run_piece(k, a + 1, 1)] if a in (-1, 3, 7, 11, 27) else
                 [run_piece(k, a, 2)] for a in range(lo, hi, 2)] for lo, hi in zip(ends, ends[1:])]

    o_parts = [[] for _ in range(O_PARTS)]

    def o_unit(part, a, runs, row, rows, col=0, cols=M):
        piece = (wo_hbm, wo_buf, (pl.ds(a, runs), pl.ds(row, rows), pl.ds(col, cols)), SEM_O + part)
        o_parts[part].append(piece)
        return [piece]

    units = []

    def sweep(lo, hi, groups):
        for k in range(lo, hi, 2):
            for first, second in zip(groups(k), groups(k + 1)):
                units.extend(first + second)

    def w_groups(k):
        first, second = run_groups(k, 0)
        if k % 32 < LATE:
            return first, second
        f = ffn_unit(k, -1, 1) + first[0][1:]
        return [f, first[0][:1], ffn_unit(k, 3, 5), first[1]], first[2:] + second

    def o_groups(k):
        part = sum(k >= cut for cut in MXU_CUTS[1:])
        lo, hi = 16 * k, 16 * k + 4 * D
        if k < LATE:
            return ([ffn_unit(k, 0, 2), o_unit(part, 0, 2, hi, 16), ffn_unit(k, 4, 6), o_unit(part, 2, 2, hi, 16)],
                    [ffn_unit(k, 1, 3), o_unit(part, 0, 2, lo, 16), ffn_unit(k, 5), o_unit(part, 2, 2, lo, 16)])
        part += max(k // 2 * 2 - MXU_CUTS[-1], 0)
        other = part + (k >= MXU_CUTS[-1])
        return ([o_unit(part, 2, 1, hi, 16), o_unit(part, 0, 2, hi, 16)],
                [o_unit(other, 0, 2, lo, 16)], [o_unit(other, 2, 2, lo, 16)])

    sweep(0, 64, w_groups)
    c0 = len(units) // 2
    c_ends = []
    for b in range(B):
        for g in range(BLOCKS):
            sweep(8 * g, 8 * g + 8, lambda k: run_groups(k, 1 + b))
            c_ends.append(len(units) // 2)
    o0 = len(units) // 2
    sweep(0, 32, o_groups)
    row = 4 * D + 16 * LATE
    for i, n in enumerate(END_UNITS):
        units.append(o_unit(ROUND_PARTS + i // 2, 3, 1, row, n))
        row += n
    queue0, queue1 = units[0::2], units[1::2]
    for i, group in enumerate(END_TINY):
        queue1 += [o_unit(O_PARTS - len(END_TINY) + i, 3, 1, row + 8 * r, 8, col, M // 2)
                   for r in group for col in (0, M // 2)]

    assert all(len(unit) == 1 for unit in queue1)

    def start(unit, queue):
        for piece in unit:
            copy(*piece).start(priority=queue)

    def issue(lo, hi):
        for i in range(lo, hi):
            start(queue0[i], 0)
            if i + LEAD < len(queue1):
                start(queue1[i + LEAD], 1)

    def issue_nth(i, ranges, first=0):
        n = len(ranges) // 2
        if n == 0:
            issue(*ranges[0])
        else:
            pl.when(i < first + n)(lambda: issue_nth(i, ranges[:n], first))
            pl.when(i >= first + n)(lambda: issue_nth(i, ranges[n:], first + n))

    issued = [2]

    def take(count, upto=0):
        issued.append(min(max(issued[-1] + count, upto), len(queue0)))
        return issued[-2:]

    x_copy, b1_copy, b2_copy, o_copy = [
        pltpu.make_async_copy(src, dst, sems.at[SEM_SMALL + i])
        for i, (src, dst) in enumerate(((x_hbm, x_buf), (b1_hbm, b1_buf), (b2_hbm, b2_buf), (o_buf, o_hbm)))]

    for i in range(LEAD + 2):
        if i in (2, 16):
            start(queue0[i // 16], 0)
        start(queue1[i], 1)
    for c in (x_copy, b1_copy, b2_copy):
        issue(*take(20))
        c.start()
    issue(*take(20))

    x_copy.wait()
    x = x_buf[...].astype(F32)
    xc = x - jnp.mean(x, axis=-1, keepdims=True)
    var = jnp.mean(xc * xc, axis=-1, keepdims=True)
    xn = xc * lax.rsqrt(var + 1e-5)

    def heads8(w_buf, h):
        return w_buf[:, :, pl.ds(h, 8)].reshape(512 * 8, D)

    def own_head(v):
        return jnp.where(lax.broadcasted_iota(jnp.int32, v.shape, 1) % 8
                         == lax.broadcasted_iota(jnp.int32, v.shape, 0) % 8, v, 0.0)

    def by_quarters(v, dims):
        n, m = v.shape[0], v.shape[1] // 4
        v = jnp.concatenate([v[:, j * m:(j + 1) * m] for j in range(4)], axis=0).astype(BF16)
        v = lax.dot_general(v, e_buf[...], dims, preferred_element_type=F32)
        return jnp.concatenate([v[j * n:(j + 1) * n] for j in range(4)], axis=1)

    e_buf[...] = (lax.broadcasted_iota(jnp.int32, (128, 1024), 1) // 8
                  == lax.broadcasted_iota(jnp.int32, (128, 1024), 0)).astype(F32).astype(BF16)
    xs = jnp.concatenate([jnp.broadcast_to(xn[b:b + 1], (8, M)) for b in range(B)], axis=0)
    xs = own_head(by_quarters(xs, NN)).astype(BF16)
    issue(*take(0, c0 + 40))

    wait_filled(wuv_buf, SEM_W)
    wait_filled(wuk_buf, SEM_W + 1)
    wait_filled(wq_buf, SEM_W + 2)
    after_qa = [take(12) for _ in range(H // 8)]

    def absorb(i):
        h = pl.multiple_of(i * 8, 8)
        q = jnp.dot(xs, heads8(wq_buf, h), preferred_element_type=F32).astype(BF16)
        r = lax.dot_general(q, heads8(wuk_buf, h), NT, preferred_element_type=F32)
        qa = by_quarters(own_head(r * (D ** -0.5 * LOG2E)), NT)
        for b in range(B):
            qa_ref[b, pl.ds(h, 8)] = qa[b * 8:(b + 1) * 8]
        issue_nth(i, after_qa)

    _loop(0, H // 8, absorb)

    before, during, ctx_before, ctx_during = [], [], [], []
    for i, end in enumerate(c_ends):
        before.append(take(8, end + (36 if end < o0 else 28)))
        during.append(take(15))
        if i % BLOCKS == BLOCKS - 1:
            ctx_before.append(take(8))
            ctx_during.append(take(10))

    def attention(b):
        m_ref[...] = jnp.full((H, 128), -jnp.inf, F32)
        l_ref[...] = jnp.zeros((H, 128), F32)
        acc_ref[...] = jnp.zeros((H, DC), F32)

        def block(g):
            i = b * BLOCKS + g
            issue_nth(i, before)
            runs, rows = pl.ds(b * C_RUNS, C_RUNS), pl.ds(pl.multiple_of(g * 128, 128), 128)
            wait_filled(c_buf.at[runs, rows], SEM_C + i)
            sc = lax.dot_general(qa_ref[b].astype(BF16), c_buf[runs, rows].reshape(C_RUNS * 128, DC), NT,
                                 preferred_element_type=F32)
            m_prev = m_ref[...]
            m_new = jnp.maximum(m_prev, jnp.max(sc, axis=1, keepdims=True))
            p = jnp.exp2(sc - m_new[:, :1])
            alpha = jnp.exp2(m_prev - m_new)
            l_ref[...] = alpha * l_ref[...] + jnp.sum(p, axis=1, keepdims=True)
            m_ref[...] = m_new
            p = p.astype(BF16)
            issue_nth(i, during)
            pv = jnp.dot(p, c_buf[runs, rows].reshape(C_RUNS * 128, DC), preferred_element_type=F32)
            acc_ref[...] = acc_ref[...] * alpha[:, :1] + pv

        _loop(0, BLOCKS, block)
        issue_nth(b, ctx_before)

        pc = own_head(by_quarters(acc_ref[...] / l_ref[...][:, :1], NN))
        ctx = []
        for h in range(0, H, 8):
            if h == H // 2:
                issue_nth(b, ctx_during)
            ctx.append(jnp.dot(pc[h:h + 8].astype(BF16), heads8(wuv_buf, h), preferred_element_type=F32))
        ctx = jnp.concatenate(ctx, axis=0).astype(BF16).astype(F32)
        ctx_ref[pl.ds(pl.multiple_of(b * H, H), H)] = ctx
        for k, h in enumerate(VPU_HEADS):
            mul_ref[b, k * D:(k + 1) * D] = jnp.broadcast_to(ctx[h:h + 1], (128, 128)).T

    _loop(0, B, attention)

    def wait_part(i):
        for piece in o_parts[i]:
            copy(*piece).wait()

    def spans(lo, hi):
        return [(h // 2, h % 2 * 4 * D + r, min(16 * hi, r // D * D + D) - r)
                for h in range(8 if lo < LATE else 7)
                for r in range(16 * lo, 16 * hi, 16) if r == 16 * lo or r % D == 0]

    groups = [spans(lo, hi) for lo, hi in zip(MXU_CUTS, MXU_CUTS[1:])]
    issue(*take(8))
    lhs = [jnp.concatenate([ctx_ref[pl.ds(a * 8 + r // D, B, stride=H), :][:, r % D:r % D + n]
                            for a, r, n in group], axis=1).astype(BF16) for group in groups]
    s = jnp.zeros((B, M), F32)
    for i, group in enumerate(groups):
        issue(*take(0, o0 + 4 * MXU_CUTS[i + 1] + 28))
        wait_part(i)
        rhs = jnp.concatenate([wo_buf[a, r:r + n] for a, r, n in group], axis=0)
        s = s + jnp.dot(lhs[i], rhs, preferred_element_type=F32)
        if MXU_CUTS[i + 1] == LATE:
            wait_filled(w1_buf, SEM_FFN)
            wait_filled(w2_buf, SEM_FFN + 1)
            b1_copy.wait()
            b2_copy.wait()
            w1 = w1_buf[...].reshape(M // 8, F // 128, 8, 128)
            w1 = jnp.concatenate([w1[:, j].reshape(M, 128) for j in range(F // 128)], axis=1)
            hid = jnp.dot(xn.astype(BF16), w1, preferred_element_type=F32) + b1_buf[...].astype(F32).reshape(1, F)
            hid = jax.nn.gelu(hid, approximate=True).astype(BF16)
            z = jnp.dot(hid, w2_buf[...], preferred_element_type=F32) + b2_buf[...].astype(F32).reshape(1, M)
            z8 = _rows8(z)
            g8 = z8 * jax.nn.sigmoid(z8)
    assert issued[-1] == len(queue0) >= len(queue1) - LEAD
    base8 = _rows8(x) + _rows8(s) * g8

    sublane = lax.broadcasted_iota(jnp.int32, (8, 128), 0)
    upper = {k: (sublane & k) != 0 for k in (1, 2, 4)}
    part, terms = None, None
    for i in range(len(groups), O_PARTS):
        wait_part(i)
        for _, _, (runs, rows, cols), _ in o_parts[i]:
            if cols.start:
                continue
            for a in range(runs.start, runs.start + runs.size):
                for r in range(rows.start, rows.start + rows.size, 8):
                    w = wo_buf[a, r:r + 8].astype(F32)
                    part = terms if part is None else [p + t for p, t in zip(part, terms)]
                    at = pl.ds(VPU_HEADS.index(a * 8 + r // D) * D + r % D, 8)
                    mul = [mul_ref[b, at, :] for b in range(B)]
                    terms = [w[:, j * 128:(j + 1) * 128] * mul[b] for j in range(M // 128) for b in range(B)]
    part = [p + t for p, t in zip(part, terms)]

    part = [jnp.where(upper[4], hi, lo) + pltpu.roll(jnp.where(upper[4], lo, hi), 4, 0)
            for lo, hi in zip(part[:4], part[4:])]
    for k in (2, 1):
        part = [jnp.where(upper[k], hi, lo) + jnp.where(upper[k], pltpu.roll(hi, k, 0), pltpu.roll(lo, 8 - k, 0))
                for lo, hi in zip(part[:k], part[k:])]
    o_buf[...] = (base8 + g8 * part[0]).astype(BF16)
    o_copy.start()
    o_copy.wait()


@jax.jit
def pallas_recurrent_scan__compressed_kv_cla__dense_activation_gelu__decode_kernel(
    A_x: jax.Array,
    A_c_kv: jax.Array,
    A_w_q: jax.Array,
    A_w_uk: jax.Array,
    A_w_uv: jax.Array,
    A_w_o: jax.Array,
    B_x: jax.Array,
    B_w1: jax.Array,
    B_b1: jax.Array,
    B_w2: jax.Array,
    B_b2: jax.Array,
):
    del B_x
    hbm = pl.BlockSpec(memory_space=pltpu.HBM)
    w1_tiles = B_w1.reshape(M // 8, 8, F // 128, 128).transpose(0, 2, 1, 3).reshape(W1_VIEW)
    out = pl.pallas_call(
        _kernel,
        out_shape=jax.ShapeDtypeStruct((8, 128), BF16),
        in_specs=[hbm] * 10,
        out_specs=hbm,
        scratch_shapes=[
            pltpu.VMEM(C_VIEW, BF16), pltpu.VMEM(W_VIEW, BF16), pltpu.VMEM(W_VIEW, BF16),
            pltpu.VMEM(W_VIEW, BF16), pltpu.VMEM(O_VIEW, BF16),
            pltpu.VMEM(W1_VIEW, BF16), pltpu.VMEM((F, M), BF16),
            pltpu.VMEM((B, H, DC), F32), pltpu.VMEM((H, DC), F32),
            pltpu.VMEM((H, 128), F32), pltpu.VMEM((H, 128), F32),
            pltpu.VMEM((128, 1024), BF16),
            pltpu.VMEM((3 * H, D), F32), pltpu.VMEM((B, len(VPU_HEADS) * D, 128), F32),
            pltpu.VMEM((8, 128), BF16),
            pltpu.VMEM((F,), BF16), pltpu.VMEM((B, M), BF16), pltpu.VMEM((M,), BF16),
            pltpu.SemaphoreType.DMA((SEM_O + O_PARTS,)),
        ],
        compiler_params=pltpu.CompilerParams(
            vmem_limit_bytes=100 * 1024 * 1024, disable_semaphore_checks=True, disable_bounds_checks=True),
    )(A_x.reshape(B, M), A_c_kv.reshape(C_VIEW), A_w_q.reshape(W_VIEW), A_w_uk.reshape(W_VIEW),
      A_w_uv.reshape(W_VIEW), A_w_o.reshape(O_VIEW), w1_tiles, B_b1, B_w2, B_b2)
    return out.reshape(M // 128, B, 128).transpose(1, 0, 2).reshape(B, 1, M)
```
